```python
import os as _os
_os.environ.setdefault("JAX_PLATFORMS", "cpu")
import jax
import jax.numpy as jnp

def _softmax(x, axis=-1):
    return jax.nn.softmax(x, axis=axis)
def _gelu(x):
    return jax.nn.gelu(x, approximate=True)
def _silu(x):
    return jax.nn.silu(x)
def _sigmoid(x):
    return jax.nn.sigmoid(x)
def _layernorm(x, axis=-1, eps=1e-5):
    m = jnp.mean(x, axis=axis, keepdims=True)
    v = jnp.var(x, axis=axis, keepdims=True)
    return (x - m) / jnp.sqrt(v + eps)
def _scatter_add(tgt, idx, src, axis=0):
    return tgt.at[idx].add(src)
def _segment_sum(src, seg, n):
    return jax.ops.segment_sum(src, seg, n)
class _Rng:
    def __init__(self, key):
        self._k = key
    def _next(self):
        self._k, sub = jax.random.split(self._k)
        return sub
    def normal(self, shape):
        return jax.random.normal(self._next(), shape, dtype=jnp.bfloat16)
    def randint(self, lo, hi, shape):
        return jax.random.randint(self._next(), shape, lo, hi, dtype=jnp.int32)
    def uniform(self, shape, lo=0.0, hi=1.0):
        return jax.random.uniform(self._next(), shape, jnp.bfloat16, lo, hi)
    def permutation(self, n):
        return jax.random.permutation(self._next(), n)


kernel_name = 'concat_heads__sliding_local_dilated__linear_attn_block__prompt'

def setup_inputs():
    _rng = _Rng(jax.random.key(int.from_bytes(__import__("os").urandom(4), "little")))
    _w = (lambda a: (lambda t: t.astype(jnp.bfloat16) if jnp.issubdtype(t.dtype, jnp.floating) else t)(jnp.asarray(a)))
    def _A_setup():
        B, S, D = 1, 2048, 640
        return {
            "x": _w((lambda *s: _rng.normal(s) * 0.2)(B, S, D)),
            "wqkv": _w((lambda *s: _rng.normal(s) * 0.2)(D, 3 * D)),
            "wo": _w((lambda *s: _rng.normal(s) * 0.05)(D, D)),
        }
    _A_in = _A_setup()

    def _B_setup():
        B, S, D = 1, 2048, 640
        return {
            "x": _w((lambda *s: _rng.normal(s) * 0.05)(B, S, D)),
            "wqkv": _w((lambda *s: _rng.normal(s) * 1.6)(D, 3 * D)),
            "wo": _w((lambda *s: _rng.normal(s) * 0.4)(D, D)),
        }
    _B_in = _B_setup()

    return {
        "A_x": _A_in["x"],
        "A_wqkv": _A_in["wqkv"],
        "A_wo": _A_in["wo"],
        "B_x": _B_in["x"],
        "B_wqkv": _B_in["wqkv"],
        "B_wo": _B_in["wo"],
    }

def reference(A_x, A_wqkv, A_wo, B_x, B_wqkv, B_wo):
    def _A_ref(x, wqkv, wo):
        B, S, D = x.shape
        H = 32; Dh = D // H
        W, dil = 8, 2
        qkv = (lambda x, *d: x.transpose(*d))((x @ wqkv).reshape(B, S, 3, H, Dh), 2, 0, 3, 1, 4)
        q, k, v = qkv[0], qkv[1], qkv[2]
        scale = Dh ** -0.5
        pos = jnp.arange(S)
        off = jnp.arange(W) * dil
        idx = pos[:, None] - off[None, :]
        mask = idx >= 0
        idx_c = jnp.where(mask, idx, 0).reshape(-1)
        kg = k[:, :, idx_c, :].reshape(B, H, S, W, Dh)
        vg = v[:, :, idx_c, :].reshape(B, H, S, W, Dh)
        logits = jnp.einsum("bhsd,bhswd->bhsw", q, kg) * scale
        logits = jnp.where(mask[None, None, :, :], logits, -1e9)
        attn = _softmax(logits, axis=-1)
        o = jnp.einsum("bhsw,bhswd->bhsd", attn, vg)
        return (lambda x, *d: x.transpose(*d))(o, 0, 2, 1, 3).reshape(B, S, D) @ wo

    def _B_ref(x, wqkv, wo):
        B, S, D = x.shape
        H = 32; Dh = D // H
        qkv = (lambda x, *d: x.transpose(*d))((x @ wqkv).reshape(B, S, 3, H, Dh), 2, 0, 3, 1, 4)
        q, k, v = qkv[0], qkv[1], qkv[2]
        phi = lambda t: jnp.where(t > 0, t + 1, jnp.exp(t)) + 1e-6
        pq, pk = phi(q), phi(k)
        kv = jnp.einsum("bhsd,bhse->bhde", pk, v)
        z = jnp.einsum("bhsd->bhd", pk)
        num = jnp.einsum("bhqd,bhde->bhqe", pq, kv)
        den = jnp.einsum("bhqd,bhd->bhq", pq, z)[..., None] + 1e-6
        o = num / den
        return (lambda x, *d: x.transpose(*d))(o, 0, 2, 1, 3).reshape(B, S, D) @ wo

    a = _A_ref(A_x, A_wqkv, A_wo)
    b = _B_ref(B_x, B_wqkv, B_wo)
    return jnp.concatenate([a, b], axis=-1)
```

```python
import functools
import math

import jax
import jax.numpy as jnp
from jax import lax
import jax.experimental.pallas as pl
import jax.experimental.pallas.tpu as pltpu

S = 2048
D = 640
H = 32
DH = D // H
NT = D // 128
WIN = 8
DIL = 2
HALO = 16
BS1 = 512
NB1 = S // BS1
BS2 = 256
NB2 = S // BS2
RC = 16

F32 = jnp.float32
BF16 = jnp.bfloat16
SCALE = DH ** -0.5
EXP2_C = SCALE * math.log2(math.e)
NEG = -1e9 / SCALE

_NT_DIMS = (((1,), (1,)), ((), ()))


def _dot(a, b):
    return jnp.dot(a, b, preferred_element_type=F32)


def _dot_nt(a, b):
    return lax.dot_general(a, b, _NT_DIMS, preferred_element_type=F32)


def _phi(t):
    return jnp.where(t > 0, t + 1.0, jnp.exp(t)) + 1e-6


def _group_sum(p):
    p = p + pltpu.roll(p, 64, 1)
    return p + pltpu.roll(p, 32, 1)


_BANDS = []
for _j in range(NT):
    _h0 = (128 * _j) // DH
    _h1 = (128 * _j + 127) // DH
    _BANDS.append(((_h0 * DH) // 16 * 16, -((-(_h1 + 1) * DH) // 16) * 16))


def _kernel(xa_hbm, wa_hbm, woa_hbm, xb_hbm, wb_hbm, wob_hbm, out_hbm,
            xa, xb, wraw, wT, wkT, woaP, mP, tscr, g_s, zacc, zrow,
            q_s, k_s, v_s, qb_s, o_s, a_s, out_s,
            sem_xa, sem_xb, sem_w, sem_out):
    w_src = [
        wb_hbm.at[:, D:2 * D], wa_hbm.at[:, 0:D], wa_hbm.at[:, D:2 * D],
        wa_hbm.at[:, 2 * D:3 * D], wb_hbm.at[:, 0:D], wb_hbm.at[:, 2 * D:3 * D],
        wob_hbm, woa_hbm,
    ]

    def w_copy(i):
        return pltpu.make_async_copy(w_src[i], wraw.at[i], sem_w.at[i])

    def xb_copy(i):
        rows = pl.ds(i * BS1, BS1)
        return pltpu.make_async_copy(xb_hbm.at[rows], xb.at[rows], sem_xb.at[i])

    def xa_copy(i):
        rows = pl.ds(i * BS2, BS2)
        return pltpu.make_async_copy(xa_hbm.at[rows], xa.at[rows], sem_xa.at[i])

    def out_copy(i):
        rows = pl.ds(i * BS2, BS2)
        return pltpu.make_async_copy(out_s.at[rows], out_hbm.at[rows], sem_out.at[i])

    def permute_rows(j, dst):
        for d in range(DH):
            rows = tscr[j, pl.ds(d, H, stride=DH), :]
            dst[H * d:H * (d + 1), 128 * j:128 * (j + 1)] = rows.astype(BF16)

    def prep_transposed(src, dst):
        for j in range(NT):
            tscr[j] = src[128 * j:128 * (j + 1), :].T.astype(F32)
            permute_rows(j, dst)

    w_copy(0).start()
    xb_copy(0).start()
    xb_copy(1).start()
    w_copy(1).start()
    w_copy(0).wait()
    for j in range(NT):
        wkT[:, 128 * j:128 * (j + 1)] = wraw[0, 128 * j:128 * (j + 1), :].T
    k_s[:, BS2:BS2 + HALO, :] = jnp.zeros((NT, HALO, 128), F32)
    v_s[:, BS2:BS2 + HALO, :] = jnp.zeros((NT, HALO, 128), F32)

    for i in range(NB1):
        xb_copy(i).wait()
        if i >= 1:
            w_copy(i).wait()
        if i + 2 < NB1:
            xb_copy(i + 2).start()
        if i + 2 <= 3:
            w_copy(i + 2).start()
        if i == 2:
            for s in (4, 5, 6, 7):
                w_copy(s).start()
        if i == 3:
            for s in range(NB2):
                xa_copy(s).start()
        xblk = xb[i * BS1:(i + 1) * BS1, :]
        pkT = _phi(_dot_nt(wkT[...], xblk))
        zp = pkT[:, 0:128]
        for t in range(1, BS1 // 128):
            zp = zp + pkT[:, 128 * t:128 * (t + 1)]
        gi = _dot(pkT.astype(BF16), xblk)
        if i == 0:
            zacc[...] = zp
            g_s[...] = gi
        else:
            zacc[...] += zp
            g_s[...] += gi
        if i >= 1:
            prep_transposed(wraw.at[i], wT.at[i - 1])

    for s in (4, 5, 6, 7):
        w_copy(s).wait()
    prep_transposed(wraw.at[4], wT.at[3])
    for j in range(NT):
        tscr[j] = wraw[7, :, 128 * j:128 * (j + 1)].astype(F32)
        permute_rows(j, woaP)
    for d in range(DH):
        tscr[0, H * d:H * (d + 1), :] = zacc[pl.ds(d, H, stride=DH), :]
    for t in range(NT):
        zt = jnp.sum(tscr[0, 128 * t:128 * (t + 1), :].T, axis=0, keepdims=True)
        zrow[:, 128 * t:128 * (t + 1)] = jnp.broadcast_to(zt, (8, 128))
    tscr[...] = jnp.zeros(tscr.shape, F32)
    for j, (lo, hi) in enumerate(_BANDS):
        gb = g_s[lo:hi, :].astype(BF16)
        kv = _dot(gb, wraw[5, :, 128 * j:128 * (j + 1)])
        rh = (lax.broadcasted_iota(jnp.int32, kv.shape, 0) + lo) // DH
        ch = (lax.broadcasted_iota(jnp.int32, kv.shape, 1) + 128 * j) // DH
        kv = jnp.where(rh == ch, kv, 0.0).astype(BF16)
        mj = _dot(kv, wraw[6, 128 * j:128 * (j + 1), :])
        for t in range(NT):
            tscr[t, lo:hi, :] += mj[:, 128 * t:128 * (t + 1)]
    for j in range(NT):
        permute_rows(j, mP)

    def block(i, carry):
        r0 = pl.multiple_of(i * BS2, BS2)
        xa_copy(i).wait()
        xablk = xa[pl.ds(r0, BS2), :]
        k_tail = k_s[:, BS2:BS2 + HALO, :]
        v_tail = v_s[:, BS2:BS2 + HALO, :]
        q = _dot_nt(xablk, wT[0])
        k = _dot_nt(xablk, wT[1])
        v = _dot_nt(xablk, wT[2])
        k_s[:, 0:HALO, :] = k_tail
        for t in range(NT):
            q_s[t] = q[:, 128 * t:128 * (t + 1)]
            k_s[t, HALO:HALO + BS2, :] = k[:, 128 * t:128 * (t + 1)]
            vt = v[:, 128 * t:128 * (t + 1)]
            v_s[t, HALO:HALO + BS2, :] = vt
            v_s[t, 0:HALO, :] = jnp.where(
                i == 0, jnp.broadcast_to(vt[0:1, :], (HALO, 128)), v_tail[t])

        qb = _dot_nt(xb[pl.ds(r0, BS2), :], wT[3])
        for t in range(NT):
            qb_s[t] = qb[:, 128 * t:128 * (t + 1)]

        for c in range(BS2 // RC):
            rs = slice(c * RC, (c + 1) * RC)
            pq = [_phi(qb_s[t, rs, :]) for t in range(NT)]
            den = pq[0] * zrow[0:1, 0:128]
            for t in range(1, NT):
                den = den + pq[t] * zrow[0:1, 128 * t:128 * (t + 1)]
            rec = 1.0 / (_group_sum(den) + 1e-6)
            for t in range(NT):
                a_s[rs, 128 * t:128 * (t + 1)] = (pq[t] * rec).astype(BF16)
        out_s[pl.ds(r0, BS2), D:2 * D] = _dot(a_s[...], mP[...]).astype(BF16)

        for c in range(BS2 // RC):
            base = c * RC
            qq = [q_s[t, base:base + RC, :] for t in range(NT)]
            logits = []
            for w in range(WIN):
                off = HALO + base - DIL * w
                p = qq[0] * k_s[0, off:off + RC, :]
                for t in range(1, NT):
                    p = p + qq[t] * k_s[t, off:off + RC, :]
                p = _group_sum(p)
                if base < (WIN - 1) * DIL and w > 0:
                    grow = lax.broadcasted_iota(jnp.int32, p.shape, 0) + (r0 + base)
                    p = jnp.where(grow >= DIL * w, p, NEG)
                logits.append(p)
            m = logits[0]
            for w in range(1, WIN):
                m = jnp.maximum(m, logits[w])
            e = [jnp.exp2((logits[w] - m) * EXP2_C) for w in range(WIN)]
            tot = e[0]
            for w in range(1, WIN):
                tot = tot + e[w]
            rec = 1.0 / tot
            for t in range(NT):
                off = HALO + base
                acc = e[0] * v_s[t, off:off + RC, :]
                for w in range(1, WIN):
                    off = HALO + base - DIL * w
                    acc = acc + e[w] * v_s[t, off:off + RC, :]
                o_s[base:base + RC, 128 * t:128 * (t + 1)] = (acc * rec).astype(BF16)
        out_s[pl.ds(r0, BS2), 0:D] = _dot(o_s[...], woaP[...]).astype(BF16)
        out_copy(i).start()
        return carry

    lax.fori_loop(0, NB2, block, 0)
    for i in range(NB2):
        out_copy(i).wait()


@jax.jit
def pallas_concat_heads__sliding_local_dilated__linear_attn_block__prompt_kernel(A_x, A_wqkv, A_wo, B_x, B_wqkv, B_wo):
    any_spec = pl.BlockSpec(memory_space=pl.ANY)
    out = pl.pallas_call(
        _kernel,
        out_shape=jax.ShapeDtypeStruct((S, 2 * D), BF16),
        in_specs=[any_spec] * 6,
        out_specs=any_spec,
        scratch_shapes=[
            pltpu.VMEM((S, D), BF16),
            pltpu.VMEM((S, D), BF16),
            pltpu.VMEM((8, D, D), BF16),
            pltpu.VMEM((4, D, D), BF16),
            pltpu.VMEM((D, D), BF16),
            pltpu.VMEM((D, D), BF16),
            pltpu.VMEM((D, D), BF16),
            pltpu.VMEM((NT, D, 128), F32),
            pltpu.VMEM((D, D), F32),
            pltpu.VMEM((D, 128), F32),
            pltpu.VMEM((8, D), F32),
            pltpu.VMEM((NT, BS2, 128), F32),
            pltpu.VMEM((NT, HALO + BS2, 128), F32),
            pltpu.VMEM((NT, HALO + BS2, 128), F32),
            pltpu.VMEM((NT, BS2, 128), F32),
            pltpu.VMEM((BS2, D), BF16),
            pltpu.VMEM((BS2, D), BF16),
            pltpu.VMEM((S, 2 * D), BF16),
            pltpu.SemaphoreType.DMA((NB2,)),
            pltpu.SemaphoreType.DMA((NB1,)),
            pltpu.SemaphoreType.DMA((8,)),
            pltpu.SemaphoreType.DMA((NB2,)),
        ],
        compiler_params=pltpu.CompilerParams(vmem_limit_bytes=100 * 1024 * 1024),
    )(A_x.reshape(S, D), A_wqkv, A_wo, B_x.reshape(S, D), B_wqkv, B_wo)
    return out.reshape(1, S, 2 * D)
```

```python
import collections
import functools
import math

import jax
import jax.numpy as jnp
from jax import lax
import jax.experimental.pallas as pl
import jax.experimental.pallas.tpu as pltpu

S = 2048
D = 640
H = 32
DH = D // H
NT = D // 128
WIN = 8
DIL = 2
HALO = 16
SEG0 = 256
SEG = (S - SEG0) // 2
SEGS = (0, SEG0, SEG0 + SEG, S)
BS = 256
NB = S // BS
NG = BS // 8
PAD = 8
ATT_MARGIN = 2
LIN_HI = 7

F32 = jnp.float32
BF16 = jnp.bfloat16
U32 = jnp.uint32
SCALE = DH ** -0.5
EXP2_C = SCALE * math.log2(math.e)
NEG = -1e9 * math.log2(math.e)

_NT_DIMS = (((1,), (1,)), ((), ()))


def _dot(a, b):
    return jnp.dot(a, b, preferred_element_type=F32)


def _dot_nt(a, b):
    return lax.dot_general(a, b, _NT_DIMS, preferred_element_type=F32)


def _phi(t):
    return jnp.where(t > 0, t + 1.0, jnp.exp(t)) + 1e-6


def _recip(x):
    r = pl.reciprocal(x, approx=True)
    return r * (2.0 - x * r)


def _tree(fn, xs):
    xs = list(xs)
    while len(xs) > 1:
        xs = [fn(xs[j], xs[j + 1]) if j + 1 < len(xs) else xs[j]
              for j in range(0, len(xs), 2)]
    return xs[0]


def _group_sum(p):
    p = p + pltpu.roll(p, 64, 1)
    return p + pltpu.roll(p, 32, 1)


def _lane(t):
    return slice(128 * t, 128 * (t + 1))


def _unpack(u):
    return pltpu.bitcast(u, BF16)


def _pack(b):
    return pltpu.bitcast(b, U32)


def _pack2(lo, hi):
    return pltpu.pack_elementwise([lo, hi], packed_dtype=BF16)


def _head_of(x):
    return lax.shift_right_logical(x * 3277, 16)


_BANDS = []
for _j in range(NT):
    _h0 = (128 * _j) // DH
    _h1 = (128 * _j + 127) // DH
    _BANDS.append(((_h0 * DH) // 16 * 16, -((-(_h1 + 1) * DH) // 16) * 16))

R_KB, R_QA, R_KA, R_VA, R_QB, R_VB, R_OB, R_OA = range(8)
P_QA, P_KA, P_VA, P_QB, P_OA, P_M = range(6)


def _spread(n, lo, hi):
    return [lo + (j * (hi - lo + 1)) // n for j in range(n)]


def _kernel(xa_hbm, wa_hbm, woa_hbm, xb_hbm, wb_hbm, wob_hbm, out_hbm,
            xa, xb, wraw, wp, wkT, tscr, g_s, pk_u, zacc, ztmp, zrow,
            q_s, k0_s, k1_s, v_s, qb_s, o_s, o2_s, a_s, out_s,
            sem_wk, sem_xb, sem_w, sem_xa, sem_out, sem_tail, sem_zero):
    kb = (k0_s, k1_s)
    w_src = {
        R_QA: wa_hbm.at[:, 0:D], R_KA: wa_hbm.at[:, D:2 * D],
        R_VA: wa_hbm.at[:, 2 * D:3 * D], R_QB: wb_hbm.at[:, 0:D],
        R_VB: wb_hbm.at[:, 2 * D:3 * D], R_OB: wob_hbm, R_OA: woa_hbm,
    }

    def wk_copy(j):
        rows = pl.ds(128 * j, 128)
        return pltpu.make_async_copy(
            wb_hbm.at[rows, pl.ds(D, D)], wraw.at[R_KB, rows], sem_wk.at[j])

    def w_copy(i):
        return pltpu.make_async_copy(w_src[i], wraw.at[i], sem_w.at[i])

    def xb_copy(s):
        rows = pl.ds(SEGS[s], SEGS[s + 1] - SEGS[s])
        return pltpu.make_async_copy(xb_hbm.at[rows], xb.at[rows], sem_xb.at[s])

    def xa_copy():
        return pltpu.make_async_copy(xa_hbm, xa, sem_xa)

    def out_copy(i):
        rows = pl.ds(i * BS, BS)
        return pltpu.make_async_copy(out_s.at[rows], out_hbm.at[rows], sem_out.at[i])

    tail_copies = []

    def tail_out(i, col0, ncol):
        rows, cols = pl.ds(i * BS, BS), pl.ds(col0, ncol)
        cp = pltpu.make_async_copy(out_s.at[rows, cols], out_hbm.at[rows, cols],
                                   sem_tail.at[len(tail_copies)])
        tail_copies.append(cp)
        cp.start()

    zero = pl.semaphore_read(sem_zero)

    def gate(tok, x):
        reps = (x.shape[0] // 8, x.shape[1] // 128)
        if tok.dtype != x.dtype:
            tok = pltpu.bitcast(tok, x.dtype)
        if reps[1] > 1:
            tok = jnp.concatenate([tok] * reps[1], axis=1)
        if reps[0] > 1:
            tok = jnp.concatenate([tok] * reps[0], axis=0)
        never = jnp.full(x.shape, zero, jnp.int32) != 0
        return jnp.where(never, tok, x)

    def run_tasks(tasks, res):
        n = len(tasks)
        for j, fn in enumerate(tasks):
            row = (res.shape[0] * j // n) // 8 * 8
            fn(res[row:row + 8, 0:128])

    def t_stage(slot, raw, j, tok):
        slab = _unpack(gate(tok, _pack(wraw[raw, 128 * j:128 * (j + 1), :])))
        tscr[slot, j] = slab.T.astype(F32)

    def c_stage(slot, raw, j, tok):
        col = _unpack(gate(tok, _pack(wraw[raw, :, _lane(j)])))
        tscr[slot, j] = col.astype(F32)

    def p_stage(slot, j, half, tok):
        for d in range(half * DH // 2, (half + 1) * DH // 2):
            even = gate(tok, tscr[slot, j, pl.ds(d, H // 2, stride=DH), :])
            odd = tscr[slot, j, pl.ds(d + D // 2, H // 2, stride=DH), :]
            wp[slot, 16 * d:16 * (d + 1), _lane(j)] = _pack2(even, odd)

    def z_stage1(tok):
        for d in range(DH):
            for b in range(2):
                ztmp[pl.ds(H * d + b, H // 2, stride=2), :] = gate(
                    tok, zacc[pl.ds(d + b * D // 2, H // 2, stride=DH), :])

    def z_stage2(tok):
        for t in range(NT):
            zt = gate(tok, ztmp[128 * t:128 * (t + 1), :]).T
            zt = jnp.sum(zt, axis=0, keepdims=True)
            zrow[:, _lane(t)] = jnp.broadcast_to(zt, (8, 128))

    for j in range(NT):
        wk_copy(j).start()
    xb_copy(0).start()
    for j in range(NT):
        wk_copy(j).wait()
        wkT[:, _lane(j)] = _pack(wraw[R_KB, 128 * j:128 * (j + 1), :].T)

    def stats(lo, nrows, init, tasks):
        p = 0
        wk_val = _unpack(wkT[...])
        for n in range(nrows // 128):
            res = _dot_nt(wk_val, xb[pl.ds(lo + 128 * n, 128), :])
            pk = _phi(res)
            if init and n == 0:
                zacc[...] = pk
            else:
                zacc[...] += pk
            pk_u[:, _lane(n)] = _pack(pk.astype(BF16))
            run_tasks(tasks[p], res)
            p += 1
        pk_val = _unpack(pk_u[:, 0:nrows])
        for c in range(NT):
            res = _dot(pk_val, xb[pl.ds(lo, nrows), _lane(c)])
            if init:
                g_s[c] = res
            else:
                g_s[c] += res
            run_tasks(tasks[p], res[0:512] if c == NT - 1 else res)
            p += 1

    xb_copy(0).wait()
    xb_copy(1).start()
    xb_copy(2).start()
    for i in (R_QB, R_KA):
        w_copy(i).start()
    stats(0, SEG0, True, collections.defaultdict(list))

    def stats_step(it, carry):
        @pl.when(it == 0)
        def _():
            xb_copy(1).wait()
            for i in (R_VA, R_QA, R_VB, R_OB):
                w_copy(i).start()

        @pl.when(it == 1)
        def _():
            xb_copy(2).wait()
            for i in (R_QB, R_KA, R_VA, R_QA):
                w_copy(i).wait()
            xa_copy().start()
            w_copy(R_OA).start()

        todo = []
        for slot, raw in ((P_QB, R_QB), (P_KA, R_KA), (P_VA, R_VA), (P_QA, R_QA)):
            src = it * raw + (1 - it) * R_KB
            todo += [functools.partial(t_stage, slot, src, j) for j in range(NT)]
            todo += [functools.partial(p_stage, slot, j, hf)
                     for j in range(NT) for hf in range(2)]
        tasks = collections.defaultdict(list)
        for fn, p in zip(todo, _spread(len(todo), 0, SEG // 128 + NT - 1)):
            tasks[p].append(fn)
        stats(pl.multiple_of(SEG0 + it * SEG, 128), SEG, False, tasks)
        return carry

    lax.fori_loop(0, 2, stats_step, 0)

    for i in (R_VB, R_OB, R_OA):
        w_copy(i).wait()
    xa_copy().wait()

    def rows_of(g):
        return 16 * (g // 2) + g % 2

    def lin_group(g, tok):
        rows = pl.ds(rows_of(g), 8, stride=2)
        pq = [_phi(gate(tok, qb_s[t, rows, :])) for t in range(NT)]
        den = _tree(jnp.add, [pq[t] * zrow[:, _lane(t)] for t in range(NT)])
        rec = _recip(_group_sum(den) + 1e-6)
        for t in range(NT):
            a_s[t, rows, :] = pq[t] * rec

    def att_group(k_s, o_dst, first, g, tok):
        s0 = rows_of(g)
        cvec = gate(tok, jnp.full((8, 128), EXP2_C, F32))
        qq = [q_s[t, pl.ds(s0, 8, stride=2), :] * cvec for t in range(NT)]
        logits = []
        for w in range(WIN):
            rows = pl.ds(HALO + s0 - DIL * w, 8, stride=2)
            p = _tree(jnp.add, [qq[t] * k_s[t, rows, :] for t in range(NT)])
            p = _group_sum(p)
            if first is not None and s0 < DIL * w:
                pos = 2 * lax.broadcasted_iota(jnp.int32, p.shape, 0) + (s0 + first)
                p = jnp.where(pos >= DIL * w, p, NEG)
            logits.append(p)
        m = _tree(jnp.maximum, logits)
        e = [jnp.exp2(logits[w] - m) for w in range(WIN)]
        rec = _recip(_tree(jnp.add, e))
        for t in range(NT):
            acc = _tree(jnp.add, [
                e[w] * v_s[t, pl.ds(HALO + s0 - DIL * w, 8, stride=2), :]
                for w in range(WIN)])
            o_dst[t, pl.ds(s0, 8, stride=2), :] = acc * rec

    def packed_lhs(src):
        cols = [_pack2(src[t, pl.ds(0, BS // 2, stride=2), :],
                       src[t, pl.ds(1, BS // 2, stride=2), :]) for t in range(NT)]
        return _unpack(jnp.concatenate(cols, axis=1))

    def run_units(units, tasks, after=None):
        lhs = {}
        kvs = {}
        p = 0
        for u, (kind, i, opt) in enumerate(units):
            if isinstance(i, int):
                rows = pl.ds(i * BS, BS)
            else:
                rows = pl.ds(pl.multiple_of(i * BS, BS), BS)
            for t in range(NT):
                prow = slice(64 * t, 64 * (t + 1))
                if kind == "KV":
                    lo, hi = _BANDS[t]
                    half = (hi - lo) // 2
                    gb = _unpack(jnp.concatenate(
                        [_pack2(g_s[c, pl.ds(lo, half, stride=2), :],
                                g_s[c, pl.ds(lo + 1, half, stride=2), :])
                         for c in range(NT)], axis=1))
                    res = _dot(gb, wraw[R_VB, :, _lane(t)])
                    rh = _head_of(lax.broadcasted_iota(jnp.int32, res.shape, 0) + lo)
                    ch = _head_of(lax.broadcasted_iota(jnp.int32, res.shape, 1) + 128 * t)
                    kvs[t] = jnp.where(rh == ch, res, 0.0).astype(BF16)
                elif kind == "M":
                    lo, hi = _BANDS[t]
                    mid = _BANDS[t - 1][1] if t else lo
                    res = _dot(kvs[t], wraw[R_OB, 128 * t:128 * (t + 1), :])
                    for c in range(NT):
                        if mid > lo:
                            tscr[P_M, c, lo:mid, :] += res[0:mid - lo, _lane(c)]
                        tscr[P_M, c, mid:hi, :] = res[mid - lo:hi - lo, _lane(c)]
                elif kind in ("Q", "K", "V"):
                    key = ("xa", opt["tag"])
                    if key not in lhs:
                        lhs[key] = xa[rows, :]
                    slot = {"Q": P_QA, "K": P_KA, "V": P_VA}[kind]
                    if kind == "K":
                        k_s = kb[opt["par"]]
                        if opt.get("zero_halo"):
                            v_s[t, BS:BS + HALO, :] = jnp.zeros((HALO, 128), F32)
                            halo = jnp.zeros((HALO, 128), F32)
                        else:
                            halo = kb[1 - opt["par"]][t, BS:BS + HALO, :]
                        k_s[t, 0:HALO, :] = halo
                    if kind == "V":
                        v_tail = v_s[t, BS:BS + HALO, :]
                    res = _dot_nt(lhs[key], _unpack(wp[slot, prow, :]))
                    if kind == "Q":
                        q_s[t, 0:BS, :] = res
                    elif kind == "K":
                        k_s[t, HALO:HALO + BS, :] = res
                    else:
                        v_s[t, HALO:HALO + BS, :] = res
                        if opt.get("first") is not None:
                            v_tail = jnp.where(
                                opt["first"] == 0,
                                jnp.broadcast_to(res[0:1, :], (HALO, 128)), v_tail)
                        v_s[t, 0:HALO, :] = v_tail
                elif kind == "Bq":
                    if t == 0:
                        lhs["xb"] = xb[rows, :]
                    res = _dot_nt(lhs["xb"], _unpack(wp[P_QB, prow, :]))
                    qb_s[t, 0:BS, :] = res
                else:
                    slot, col0 = (P_M, D) if kind == "Bo" else (P_OA, 0)
                    if t == 0:
                        lhs["o"] = packed_lhs(a_s if kind == "Bo" else opt.get("o", o_s))
                    res = _dot(lhs["o"], _unpack(wp[slot, :, _lane(t)]))
                    out_s[rows, col0 + 128 * t:col0 + 128 * (t + 1)] = res.astype(BF16)
                if after is not None:
                    after(u, t)
                run_tasks(tasks[p], res)
                p += 1

    def add_groups(tasks, fn, lo, hi):
        for g, p in enumerate(_spread(NG, lo, hi)):
            tasks[p].append(functools.partial(fn, g))

    def std_units(i, par, first=None):
        opt = dict(tag=(par, 0), first=first)
        return [("V", i, opt), ("Q", i, opt),
                ("K", i + 1, dict(tag=(par, 1), par=1 - par)),
                ("Bq", i + 1, {}), ("Bo", i, {}), ("Ao", i, {})]

    def std_tasks(tasks, base, par, first=None, lin_lo=0):
        add_groups(tasks, lin_group, base + lin_lo, base + LIN_HI)
        add_groups(tasks, functools.partial(att_group, kb[par], o_s, first),
                   base + 10, base + 25 - ATT_MARGIN)

    def pair_after(i0, off):
        def after(u, t):
            if t == NT - 1 and u >= off and (u - off) % 6 == 5:
                out_copy(i0 + (u - off) // 6).start()
        return after

    tasks = collections.defaultdict(list)
    tasks[0].append(z_stage1)
    tasks[5].append(z_stage2)
    for j in range(NT):
        tasks[j].append(functools.partial(c_stage, P_OA, R_OA, j))
        for hf in range(2):
            tasks[5 + j].append(functools.partial(p_stage, P_OA, j, hf))
            tasks[15 + j].append(functools.partial(p_stage, P_M, j, hf))
    run_units([("KV", 0, {}), ("Bq", 0, {}), ("M", 0, {}),
               ("K", 0, dict(tag=(0, 0), par=0, zero_halo=True))], tasks)

    def pair(j, carry):
        tasks = collections.defaultdict(list)
        std_tasks(tasks, 0, 0, first=2 * BS * j)
        std_tasks(tasks, 30, 1, lin_lo=-5)
        run_units(std_units(2 * j, 0, first=2 * BS * j) + std_units(2 * j + 1, 1),
                  tasks, pair_after(2 * j, 0))
        return carry

    lax.fori_loop(0, NB // 2 - 1, pair, 0)

    a, b = NB - 2, NB - 1
    ob = dict(tag=(0, 1))
    units = std_units(a, 0)[:5] + [
        ("V", b, ob), ("Q", b, ob), ("Ao", a, {}), ("Bo", b, {}), ("Ao", b, dict(o=o2_s))]
    tasks = collections.defaultdict(list)
    std_tasks(tasks, 0, 0)
    add_groups(tasks, lin_group, 25, 33)
    add_groups(tasks, functools.partial(att_group, kb[1], o2_s, None), 35, 45 - ATT_MARGIN)

    def tail_after(u, t):
        if u == 9:
            tail_out(b, 128 * t, 128)
        elif t == NT - 1 and u == 7:
            out_copy(a).start()
        elif t == NT - 1 and u == 8:
            tail_out(b, D, D)

    run_units(units, tasks, tail_after)

    for i in range(NB - 1):
        out_copy(i).wait()
    for cp in tail_copies:
        cp.wait()


@jax.jit
def pallas_concat_heads__sliding_local_dilated__linear_attn_block__prompt_kernel(A_x, A_wqkv, A_wo, B_x, B_wqkv, B_wo):
    any_spec = pl.BlockSpec(memory_space=pl.ANY)
    slab = lambda rows: pltpu.VMEM((NT, rows + PAD, 128), F32)
    out = pl.pallas_call(
        _kernel,
        out_shape=jax.ShapeDtypeStruct((S, 2 * D), BF16),
        in_specs=[any_spec] * 6,
        out_specs=any_spec,
        scratch_shapes=[
            pltpu.VMEM((S, D), BF16),
            pltpu.VMEM((S, D), BF16),
            pltpu.VMEM((8, D, D), BF16),
            pltpu.VMEM((6, D // 2, D), U32),
            pltpu.VMEM((D // 2, D), U32),
            pltpu.VMEM((6, NT, D, 128), F32),
            pltpu.VMEM((NT, D, 128), F32),
            pltpu.VMEM((D // 2, SEG), U32),
            pltpu.VMEM((D, 128), F32),
            pltpu.VMEM((D, 128), F32),
            pltpu.VMEM((8, D), F32),
            slab(BS),
            slab(HALO + BS),
            slab(HALO + BS),
            slab(HALO + BS),
            slab(BS),
            slab(BS),
            slab(BS),
            slab(BS),
            pltpu.VMEM((S, 2 * D), BF16),
            pltpu.SemaphoreType.DMA((NT,)),
            pltpu.SemaphoreType.DMA((len(SEGS) - 1,)),
            pltpu.SemaphoreType.DMA((8,)),
            pltpu.SemaphoreType.DMA(()),
            pltpu.SemaphoreType.DMA((NB - 1,)),
            pltpu.SemaphoreType.DMA((NT + 1,)),
            pltpu.SemaphoreType.REGULAR,
        ],
        compiler_params=pltpu.CompilerParams(vmem_limit_bytes=100 * 1024 * 1024),
    )(A_x.reshape(S, D), A_wqkv, A_wo, B_x.reshape(S, D), B_wqkv, B_wo)
    return out.reshape(1, S, 2 * D)
```

```python
import collections
import functools
import math

import jax
import jax.numpy as jnp
from jax import lax
import jax.experimental.pallas as pl
import jax.experimental.pallas.tpu as pltpu

S = 2048
D = 640
H = 32
DH = D // H
NT = D // 128
WIN = 8
DIL = 2
HALO = 16
SEG0 = 256
SEG = (S - SEG0) // 2
SEGS = (0, SEG0, SEG0 + SEG, S)
BS = 256
NB = S // BS
NG = BS // 8
PAD = 24
SKEW = (0, 1, 0, 1, 0)

F32 = jnp.float32
BF16 = jnp.bfloat16
U32 = jnp.uint32
LOG2E = math.log2(math.e)
EXP2_C = DH ** -0.5 * LOG2E
NEG = -1e9 * LOG2E

R_KB, R_QA, R_KA, R_VA, R_QB, R_VB, R_OB, R_OA = range(8)
P_QA, P_KA, P_VA, P_QB, P_OA, P_M = range(6)

_BANDS = [(((128 * j) // DH * DH) // 16 * 16,
           -((-((128 * j + 127) // DH + 1) * DH) // 16) * 16) for j in range(NT)]


def _dot(a, b):
    return jnp.dot(a, b, preferred_element_type=F32)


def _dot_nt(a, b):
    return lax.dot_general(a, b, (((1,), (1,)), ((), ())), preferred_element_type=F32)


def _phi(t):
    return jnp.where(t > 0, t + 1.0, jnp.exp(t)) + 1e-6


def _recip(x):
    r = pl.reciprocal(x, approx=True)
    return r * (2.0 - x * r)


def _tree(fn, xs):
    xs = list(xs)
    while len(xs) > 1:
        xs = [fn(xs[j], xs[j + 1]) if j + 1 < len(xs) else xs[j]
              for j in range(0, len(xs), 2)]
    return xs[0]


def _group_sum(p):
    p = p + pltpu.roll(p, 64, 1)
    return p + pltpu.roll(p, 32, 1)


def _lane(t):
    return slice(128 * t, 128 * (t + 1))


def _unpack(u):
    return pltpu.bitcast(u, BF16)


def _pack(b):
    return pltpu.bitcast(b, U32)


def _head_of(x):
    return lax.shift_right_logical(x * 3277, 16)


def _spread(n, lo, hi):
    return [lo + (j * (hi - lo + 1)) // n for j in range(n)]


def _kernel(xa_hbm, wa_hbm, woa_hbm, xb_hbm, wb_hbm, wob_hbm, out_hbm,
            xa, xb, wraw, wp, wkT, tu, g_s, pk_u, zacc, ztmp, zrow,
            q_s, k0_s, k1_s, v0_s, v1_s, qb_s, o0_s, o1_s, a0_s, a1_s, out_s,
            sems):
    kb, vb, ob, ab = (k0_s, k1_s), (v0_s, v1_s), (o0_s, o1_s), (a0_s, a1_s)

    w_src = {
        R_QA: wa_hbm.at[:, 0:D], R_KA: wa_hbm.at[:, D:2 * D],
        R_VA: wa_hbm.at[:, 2 * D:3 * D], R_QB: wb_hbm.at[:, 0:D],
        R_VB: wb_hbm.at[:, 2 * D:3 * D], R_OB: wob_hbm, R_OA: woa_hbm,
    }

    def wk_copy(j):
        rows = pl.ds(128 * j, 128)
        return pltpu.make_async_copy(
            wb_hbm.at[rows, pl.ds(D, D)], wraw.at[R_KB, rows], sems.at[j // 3])

    def w_copy(i):
        sem = sems.at[2 if i in (R_VB, R_OB) else 1]
        return pltpu.make_async_copy(w_src[i], wraw.at[i], sem)

    def xb_copy(s):
        rows = pl.ds(SEGS[s], SEGS[s + 1] - SEGS[s])
        return pltpu.make_async_copy(xb_hbm.at[rows], xb.at[rows], sems.at[(2, 0, 1)[s]])

    def xa_copy():
        return pltpu.make_async_copy(xa_hbm, xa, sems.at[2])

    def out_copy(i, col0, ncol):
        rows, cols = pl.ds(i * BS, BS), pl.ds(col0, ncol)
        return pltpu.make_async_copy(out_s.at[rows, cols], out_hbm.at[rows, cols],
                                     sems.at[0])

    zero = [None]

    def set_zero(i):
        zero[0] = lax.shift_right_logical(i, 8)

    def gate(tok, x):
        reps = (x.shape[0] // 8, x.shape[1] // 128)
        if tok.dtype != x.dtype:
            tok = pltpu.bitcast(tok, x.dtype)
        if reps[1] > 1:
            tok = jnp.concatenate([tok] * reps[1], axis=1)
        if reps[0] > 1:
            tok = jnp.concatenate([tok] * reps[0], axis=0)
        never = jnp.full(x.shape, zero[0], jnp.int32) != 0
        return jnp.where(never, tok, x)

    def run_tasks(tasks, res):
        n = len(tasks)
        for j, fn in enumerate(tasks):
            row = (res.shape[0] * j // n) // 8 * 8
            fn(res[row:row + 8, 0:128])

    def t_stage(slot, raw, j, tok):
        slab = _unpack(gate(tok, _pack(wraw[raw, 128 * j:128 * (j + 1), :])))
        tu[slot, j] = _pack(slab.T)

    def c_stage(slot, raw, j, tok):
        tu[slot, j] = gate(tok, _pack(wraw[raw, :, _lane(j)]))

    def p_stage(slot, j, half, tok):
        for e in range(half * DH // 4, (half + 1) * DH // 4):
            lo = gate(tok, tu[slot, j, pl.ds(e, H // 2, stride=DH // 2), :])
            hi = tu[slot, j, pl.ds(e + D // 4, H // 2, stride=DH // 2), :]
            wp[slot, 32 * e:32 * e + 16, _lane(j)] = (lo & 0xFFFF) | (hi << 16)
            wp[slot, 32 * e + 16:32 * e + 32, _lane(j)] = (
                (lo >> 16) | (hi & jnp.uint32(0xFFFF0000)))

    def z_stage1(tok):
        for d in range(DH):
            for b in range(2):
                ztmp[pl.ds(H * d + b, H // 2, stride=2), :] = gate(
                    tok, zacc[pl.ds(d + b * D // 2, H // 2, stride=DH), :])

    def z_stage2(tok):
        for t in range(NT):
            zt = gate(tok, ztmp[128 * t:128 * (t + 1), :]).T
            zt = jnp.sum(zt, axis=0, keepdims=True)
            zrow[:, _lane(t)] = jnp.broadcast_to(zt, (8, 128))

    for j in range(NT):
        wk_copy(j).start()
    xb_copy(0).start()
    for group in ((0, 1, 2), (3, 4)):
        for j in group:
            wk_copy(j).wait()
        for j in group:
            wkT[:, _lane(j)] = _pack(wraw[R_KB, 128 * j:128 * (j + 1), :].T)

    def stats(lo, nrows, init, tasks):
        p = 0
        wk_val = _unpack(wkT[...])
        for n in range(nrows // 128):
            res = _dot_nt(wk_val, xb[pl.ds(lo + 128 * n, 128), :])
            pk = _phi(res)
            if init and n == 0:
                zacc[...] = pk
            else:
                zacc[...] += pk
            pk_u[:, _lane(n)] = _pack(pk.astype(BF16))
            run_tasks(tasks[p], res)
            p += 1
        for k0, kn in (((0, 128), (128, nrows - 128)) if init else ((0, nrows),)):
            pk_val = _unpack(pk_u[:, k0:k0 + kn])
            for c in range(NT):
                res = _dot(pk_val, xb[pl.ds(lo + k0, kn), _lane(c)])
                if init and k0 == 0:
                    g_s[c] = res
                else:
                    g_s[c] += res
                run_tasks(tasks[p], res[0:512] if c == NT - 1 else res)
                p += 1

    xb_copy(0).wait()
    xb_copy(1).start()
    xb_copy(2).start()
    for i in (R_QB, R_KA):
        w_copy(i).start()
    stats(0, SEG0, True, collections.defaultdict(list))

    prep = ((P_QB, R_QB), (P_KA, R_KA), (P_VA, R_VA), (P_QA, R_QA), (P_OA, R_OA))

    def stats_step(it, carry):
        @pl.when(it == 0)
        def _():
            for i in (R_VA, R_QA, R_OA):
                w_copy(i).start()
            xb_copy(1).wait()

        @pl.when(it == 1)
        def _():
            for i in (R_VB, R_OB):
                w_copy(i).start()
            xa_copy().start()
            xb_copy(2).wait()
            for _, raw in prep:
                w_copy(raw).wait()

        set_zero(it)
        todo = [functools.partial(c_stage if slot == P_OA else t_stage, slot,
                                  it * raw + (1 - it) * R_KB, j)
                for slot, raw in prep for j in range(NT)]
        todo += [functools.partial(p_stage, slot, j, half)
                 for slot, _ in prep for j in range(NT) for half in range(2)]
        tasks = collections.defaultdict(list)
        room = [1.0] * (SEG // 128) + [1.5] * NT
        for n, fn in enumerate(todo):
            x, p = (n + 0.5) * sum(room) / len(todo), 0
            while x > room[p]:
                x -= room[p]
                p += 1
            tasks[p].append(fn)
        stats(pl.multiple_of(SEG0 + it * SEG, 128), SEG, False, tasks)
        return carry + it

    set_zero(lax.fori_loop(0, 2, stats_step, 0))

    for i in (R_VB, R_OB):
        w_copy(i).wait()
    xa_copy().wait()

    def bf16_rows(src, lo, hi):
        return jnp.concatenate([src[t, lo:hi, :] for t in range(NT)], axis=1).astype(BF16)

    k1_s[:, BS:BS + HALO + 8, :] = jnp.zeros((NT, HALO + 8, 128), F32)
    v1_s[:, BS:BS + HALO + 8, :] = jnp.zeros((NT, HALO + 8, 128), F32)
    kvs, carry_rows = {}, None
    for p, (kind, t) in enumerate(
            [("KV", 0), ("KV", 1), ("KV", 2), ("M", 0), ("KV", 3), ("M", 1),
             ("KV", 4), ("M", 2), ("M", 3), ("M", 4)]):
        lo, hi = _BANDS[t]
        if kind == "KV":
            res = _dot(bf16_rows(g_s, lo, hi), wraw[R_VB, :, _lane(t)])
            rh = _head_of(lax.broadcasted_iota(jnp.int32, res.shape, 0) + lo)
            ch = _head_of(lax.broadcasted_iota(jnp.int32, res.shape, 1) + 128 * t)
            kvs[t] = jnp.where(rh == ch, res, 0.0).astype(BF16)
        else:
            res = _dot(kvs[t], wraw[R_OB, 128 * t:128 * (t + 1), :])
            done = res
            if t:
                n = _BANDS[t - 1][1] - lo
                done = jnp.concatenate([res[0:n] + carry_rows, res[n:]], axis=0)
            end = _BANDS[t + 1][0] if t + 1 < NT else hi
            carry_rows = res[end - lo:]
            done = _pack(done[0:end - lo].astype(BF16))
            for c in range(NT):
                tu[P_M, c, lo // 2:end // 2, :] = done[:, _lane(c)]
        run_tasks({0: [z_stage1], 3: [z_stage2]}.get(p, []), res)

    def rows_of(g):
        return 16 * (g // 2) + g % 2

    def lin_group(par, g, tok):
        rows = pl.ds(rows_of(g), 8, stride=2)
        pq = [_phi(gate(tok, qb_s[t, rows, :])) for t in range(NT)]
        den = _tree(jnp.add, [pq[t] * zrow[:, _lane(t)] for t in range(NT)])
        rec = _recip(_group_sum(den) + 1e-6)
        for t in range(NT):
            ab[par][t, rows, :] = pq[t] * rec

    def att_group(par, row0, g, tok):
        s0 = rows_of(g)

        def tap(t, w):
            return pl.ds(SKEW[t] + HALO + s0 - DIL * w, 8, stride=2)

        cvec = gate(tok, jnp.full((8, 128), EXP2_C, F32))
        qq = [q_s[t, pl.ds(s0, 8, stride=2), :] * cvec for t in range(NT)]
        logits = []
        for w in range(WIN):
            p = _tree(jnp.add, [qq[t] * kb[par][t, tap(t, w), :] for t in range(NT)])
            p = _group_sum(p)
            if par == 0 and s0 < DIL * w:
                pos = 2 * lax.broadcasted_iota(jnp.int32, p.shape, 0) + (s0 + row0)
                p = jnp.where(pos >= DIL * w, p, NEG)
            logits.append(p)
        m = _tree(jnp.maximum, logits)
        e = [jnp.exp2(logits[w] - m) for w in range(WIN)]
        rec = _recip(_tree(jnp.add, e))
        for t in range(NT):
            acc = _tree(jnp.add, [e[w] * vb[par][t, tap(t, w), :] for w in range(WIN)])
            ob[par][t, pl.ds(s0, 8, stride=2), :] = acc * rec

    def pair(j, carry):
        set_zero(j)
        row0 = 2 * BS * j
        tasks = collections.defaultdict(list)
        for c in range(NT):
            tasks[c] += [functools.partial(p_stage, P_M, c, half) for half in range(2)]
        for fn, lo, hi in ((functools.partial(lin_group, 0), 5, 17),
                           (functools.partial(att_group, 0, row0), 20, 32),
                           (functools.partial(lin_group, 1), 33, 39),
                           (functools.partial(att_group, 1, row0), 40, 52)):
            for g, p in enumerate(_spread(NG, lo, hi)):
                tasks[p].append(functools.partial(fn, g))

        lhs = {}
        p = 0
        for kind, par in (("Bq", 0), ("K", 0), ("V", 0), ("Q", 0),
                          ("K", 1), ("Bq", 1), ("V", 1), ("Q", 1),
                          ("Bo", 0), ("Ao", 0), ("Bo", 1), ("Ao", 1)):
            blk = 2 * j + par
            rows = pl.ds(pl.multiple_of(blk * BS, BS), BS)
            src = {"Bq": "xb", "Bo": "a", "Ao": "o"}.get(kind, "xa")
            if (src, par) not in lhs:
                if src in ("xa", "xb"):
                    lhs[src, par] = (xa if src == "xa" else xb)[rows, :]
                else:
                    lhs[src, par] = bf16_rows((ab if src == "a" else ob)[par], 0, BS)
            x = lhs[src, par]
            for t in range(NT):
                halo = pl.ds(SKEW[t], HALO)
                body = pl.ds(SKEW[t] + HALO, BS)
                tail = pl.ds(SKEW[t] + BS, HALO)
                if kind in ("Bo", "Ao"):
                    slot, col0 = (P_M, D) if kind == "Bo" else (P_OA, 0)
                    res = _dot(x, _unpack(wp[slot, :, _lane(t)]))
                    out_s[rows, col0 + 128 * t:col0 + 128 * (t + 1)] = res.astype(BF16)
                    if (kind, par) == ("Ao", 0) and t == NT - 1:
                        out_copy(blk, 0, 2 * D).start()
                    elif (kind, par) == ("Bo", 1) and t == NT - 1:
                        out_copy(blk, D, D).start()
                    elif (kind, par) == ("Ao", 1) and t >= 2:
                        (out_copy(blk, 0, 384) if t == 2
                         else out_copy(blk, 128 * t, 128)).start()
                else:
                    slot = {"Q": P_QA, "K": P_KA, "V": P_VA, "Bq": P_QB}[kind]
                    if kind == "K":
                        kb[par][t, halo, :] = kb[1 - par][t, tail, :]
                    if kind == "V":
                        prev = vb[1 - par][t, tail, :]
                    res = _dot_nt(x, _unpack(wp[slot, 64 * t:64 * (t + 1), :]))
                    if kind == "Q":
                        q_s[t, 0:BS, :] = res
                    elif kind == "Bq":
                        qb_s[t, 0:BS, :] = res
                    elif kind == "K":
                        kb[par][t, body, :] = res
                    else:
                        vb[par][t, body, :] = res
                        if par == 0:
                            prev = jnp.where(
                                j == 0, jnp.broadcast_to(res[0:1, :], (HALO, 128)), prev)
                        vb[par][t, halo, :] = prev
                run_tasks(tasks[p], res)
                p += 1
        return carry

    lax.fori_loop(0, NB // 2, pair, 0)
    pltpu.make_async_copy(out_s, out_hbm, sems.at[0]).wait()


@jax.jit
def pallas_concat_heads__sliding_local_dilated__linear_attn_block__prompt_kernel(
    A_x: jax.Array,
    A_wqkv: jax.Array,
    A_wo: jax.Array,
    B_x: jax.Array,
    B_wqkv: jax.Array,
    B_wo: jax.Array,
):
    any_spec = pl.BlockSpec(memory_space=pl.ANY)
    slab = lambda rows: pltpu.VMEM((NT, rows + PAD, 128), F32)
    extra = {name: True for name in ("disable_bounds_checks", "disable_semaphore_checks")
             if hasattr(pltpu.CompilerParams, name)}
    out = pl.pallas_call(
        _kernel,
        out_shape=jax.ShapeDtypeStruct((S, 2 * D), BF16),
        in_specs=[any_spec] * 6,
        out_specs=any_spec,
        scratch_shapes=[
            pltpu.VMEM((S, D), BF16),
            pltpu.VMEM((S, D), BF16),
            pltpu.VMEM((8, D, D), BF16),
            pltpu.VMEM((6, D // 2, D), U32),
            pltpu.VMEM((D // 2, D), U32),
            pltpu.VMEM((6, NT, D // 2, 128), U32),
            pltpu.VMEM((NT, D, 128), F32),
            pltpu.VMEM((D // 2, SEG), U32),
            pltpu.VMEM((D, 128), F32),
            pltpu.VMEM((D, 128), F32),
            pltpu.VMEM((8, D), F32),
            slab(BS),
            slab(HALO + BS), slab(HALO + BS),
            slab(HALO + BS), slab(HALO + BS),
            slab(BS),
            slab(BS), slab(BS),
            slab(BS), slab(BS),
            pltpu.VMEM((S, 2 * D), BF16),
            pltpu.SemaphoreType.DMA((3,)),
        ],
        compiler_params=pltpu.CompilerParams(
            vmem_limit_bytes=64 * 1024 * 1024, **extra),
    )(A_x.reshape(S, D), A_wqkv, A_wo, B_x.reshape(S, D), B_wqkv, B_wo)
    return out.reshape(1, S, 2 * D)
```

```python
import collections
import functools
import math

import jax
import jax.numpy as jnp
from jax import lax
import jax.experimental.pallas as pl
import jax.experimental.pallas.tpu as pltpu

S = 2048
D = 640
H = 32
DH = D // H
NT = D // 128
WIN = 8
DIL = 2
HALO = 16
SEG0 = 256
SEG = (S - SEG0) // 2
SEGS = (0, SEG0, SEG0 + SEG, S)
BS = 256
NB = S // BS
NG = BS // 8
PAD = 24
SKEW = (0, 1, 0, 1, 0)

F32 = jnp.float32
BF16 = jnp.bfloat16
U32 = jnp.uint32
LOG2E = math.log2(math.e)
EXP2_C = DH ** -0.5 * LOG2E
NEG = -1e9 * LOG2E

R_KB, R_QA, R_KA, R_VA, R_QB, R_VB, R_OB, R_OA = range(8)
P_QA, P_KA, P_VA, P_QB, P_OA, P_M = range(6)

_BANDS = [(((128 * j) // DH * DH) // 16 * 16,
           -((-((128 * j + 127) // DH + 1) * DH) // 16) * 16) for j in range(NT)]


def _dot(a, b):
    return jnp.dot(a, b, preferred_element_type=F32)


def _dot_nt(a, b):
    return lax.dot_general(a, b, (((1,), (1,)), ((), ())), preferred_element_type=F32)


def _phi(t):
    return jnp.where(t > 0, t + 1.0, jnp.exp(t)) + 1e-6


def _recip(x):
    r = pl.reciprocal(x, approx=True)
    return r * (2.0 - x * r)


def _tree(fn, xs):
    xs = list(xs)
    while len(xs) > 1:
        xs = [fn(xs[j], xs[j + 1]) if j + 1 < len(xs) else xs[j]
              for j in range(0, len(xs), 2)]
    return xs[0]


def _group_sum(p):
    p = p + pltpu.roll(p, 64, 1)
    return p + pltpu.roll(p, 32, 1)


def _lane(t):
    return slice(128 * t, 128 * (t + 1))


def _unpack(u):
    return pltpu.bitcast(u, BF16)


def _pack(b):
    return pltpu.bitcast(b, U32)


def _head_of(x):
    return lax.shift_right_logical(x * 3277, 16)


def _spread(n, lo, hi):
    return [lo + (j * (hi - lo + 1)) // n for j in range(n)]


def _kernel(xa_hbm, wa_hbm, woa_hbm, xb_hbm, wb_hbm, wob_hbm, out_hbm,
            xa, xb, wraw, wp, wq0, wkT, tu, g_s, pk_u, zacc, ztmp, zrow,
            q_s, k0_s, k1_s, v0_s, v1_s, qb_s, o0_s, o1_s, a0_s, a1_s, out_s,
            sems):
    kb, vb, ob, ab = (k0_s, k1_s), (v0_s, v1_s), (o0_s, o1_s), (a0_s, a1_s)

    w_src = {
        R_QA: wa_hbm.at[:, 0:D], R_KA: wa_hbm.at[:, D:2 * D],
        R_VA: wa_hbm.at[:, 2 * D:3 * D], R_QB: wb_hbm.at[:, 0:D],
        R_VB: wb_hbm.at[:, 2 * D:3 * D], R_OB: wob_hbm, R_OA: woa_hbm,
    }

    def wk_copy(j):
        rows = pl.ds(128 * j, 128)
        return pltpu.make_async_copy(
            wb_hbm.at[rows, pl.ds(D, D)], wraw.at[R_KB, rows], sems.at[j // 3])

    def w_copy(i):
        sem = sems.at[2 if i in (R_VB, R_OB) else 1]
        return pltpu.make_async_copy(w_src[i], wraw.at[i], sem)

    def xb_copy(s):
        rows = pl.ds(SEGS[s], SEGS[s + 1] - SEGS[s])
        return pltpu.make_async_copy(xb_hbm.at[rows], xb.at[rows], sems.at[(2, 0, 1)[s]])

    def xa_copy():
        return pltpu.make_async_copy(xa_hbm, xa, sems.at[2])

    def out_copy(i, col0, ncol):
        rows, cols = pl.ds(i * BS, BS), pl.ds(col0, ncol)
        return pltpu.make_async_copy(out_s.at[rows, cols], out_hbm.at[rows, cols],
                                     sems.at[0])

    zero = [None]

    def set_zero(i):
        zero[0] = lax.shift_right_logical(i, 8)

    def gate(tok, x):
        reps = (x.shape[0] // 8, x.shape[1] // 128)
        if tok.dtype != x.dtype:
            tok = pltpu.bitcast(tok, x.dtype)
        if reps[1] > 1:
            tok = jnp.concatenate([tok] * reps[1], axis=1)
        if reps[0] > 1:
            tok = jnp.concatenate([tok] * reps[0], axis=0)
        never = jnp.full(x.shape, zero[0], jnp.int32) != 0
        return jnp.where(never, tok, x)

    def run_tasks(tasks, res):
        n = len(tasks)
        for j, fn in enumerate(tasks):
            row = (res.shape[0] * j // n) // 8 * 8
            fn(res[row:row + 8, 0:128])

    def t_stage(slot, raw, j, tok):
        slab = _unpack(gate(tok, _pack(wraw[raw, 128 * j:128 * (j + 1), :])))
        tu[slot, j] = _pack(slab.T)

    def c_stage(slot, raw, j, tok):
        tu[slot, j] = gate(tok, _pack(wraw[raw, :, _lane(j)]))

    def p_stage(slot, j, half, tok):
        for e in range(half * DH // 4, (half + 1) * DH // 4):
            lo = gate(tok, tu[slot, j, pl.ds(e, H // 2, stride=DH // 2), :])
            hi = tu[slot, j, pl.ds(e + D // 4, H // 2, stride=DH // 2), :]
            wp[slot, 32 * e:32 * e + 16, _lane(j)] = (lo & 0xFFFF) | (hi << 16)
            wp[slot, 32 * e + 16:32 * e + 32, _lane(j)] = (
                (lo >> 16) | (hi & jnp.uint32(0xFFFF0000)))

    def n_stage(tok):
        wq0[...] = _pack(_unpack(gate(tok, wp[P_QB, 0:64, :])).T)

    def z_stage1(tok):
        for d in range(DH):
            for b in range(2):
                ztmp[pl.ds(H * d + b, H // 2, stride=2), :] = gate(
                    tok, zacc[pl.ds(d + b * D // 2, H // 2, stride=DH), :])

    def z_stage2(tok):
        for t in range(NT):
            zt = gate(tok, ztmp[128 * t:128 * (t + 1), :]).T
            zt = jnp.sum(zt, axis=0, keepdims=True)
            zrow[:, _lane(t)] = jnp.broadcast_to(zt, (8, 128))

    for j in range(NT):
        wk_copy(j).start()
    xb_copy(0).start()
    for group in ((0, 1, 2), (3, 4)):
        for j in group:
            wk_copy(j).wait()
        for j in group:
            wkT[:, _lane(j)] = _pack(wraw[R_KB, 128 * j:128 * (j + 1), :].T)

    def stats(lo, nrows, init, tasks):
        p = 0
        wk_val = _unpack(wkT[...])
        for n in range(nrows // 128):
            if n == 0:
                res = _dot(xb[pl.ds(lo, 128), :], wraw[R_KB])
                pk = _phi(res).T
            else:
                res = _dot_nt(wk_val, xb[pl.ds(lo + 128 * n, 128), :])
                pk = _phi(res)
            if init and n == 0:
                zacc[...] = pk
            else:
                zacc[...] += pk
            pk_u[:, _lane(n)] = _pack(pk.astype(BF16))
            run_tasks(tasks[p], res)
            p += 1
        for k0, kn in (((0, 128), (128, nrows - 128)) if init else ((0, nrows),)):
            pk_val = _unpack(pk_u[:, k0:k0 + kn])
            for c in range(NT):
                res = _dot(pk_val, xb[pl.ds(lo + k0, kn), _lane(c)])
                if init and k0 == 0:
                    g_s[c] = res
                else:
                    g_s[c] += res
                run_tasks(tasks[p], res[0:512] if c == NT - 1 else res)
                p += 1

    xb_copy(0).wait()
    xb_copy(1).start()
    xb_copy(2).start()
    for i in (R_QB, R_KA):
        w_copy(i).start()
    stats(0, SEG0, True, collections.defaultdict(list))

    prep = ((P_QB, R_QB), (P_KA, R_KA), (P_VA, R_VA), (P_QA, R_QA), (P_OA, R_OA))

    def stats_step(it, carry):
        @pl.when(it == 0)
        def _():
            for i in (R_VA, R_QA, R_OA):
                w_copy(i).start()
            xb_copy(1).wait()

        @pl.when(it == 1)
        def _():
            for i in (R_VB, R_OB):
                w_copy(i).start()
            xa_copy().start()
            xb_copy(2).wait()
            for _, raw in prep:
                w_copy(raw).wait()

        set_zero(it)
        todo = [functools.partial(c_stage if slot == P_OA else t_stage, slot,
                                  it * raw + (1 - it) * R_KB, j)
                for slot, raw in prep for j in range(NT)]
        todo += [functools.partial(p_stage, slot, j, half)
                 for slot, _ in prep for j in range(NT) for half in range(2)]
        todo.insert(len(todo) - 20, n_stage)
        tasks = collections.defaultdict(list)
        room = [1.0] * (SEG // 128) + [1.5] * NT
        for n, fn in enumerate(todo):
            x, p = (n + 0.5) * sum(room) / len(todo), 0
            while x > room[p]:
                x -= room[p]
                p += 1
            tasks[p].append(fn)
        stats(pl.multiple_of(SEG0 + it * SEG, 128), SEG, False, tasks)
        return carry + it

    set_zero(lax.fori_loop(0, 2, stats_step, 0))

    for i in (R_VB, R_OB):
        w_copy(i).wait()
    xa_copy().wait()

    def bf16_rows(src, lo, hi):
        return jnp.concatenate([src[t, lo:hi, :] for t in range(NT)], axis=1).astype(BF16)

    k1_s[:, BS:BS + HALO + 8, :] = jnp.zeros((NT, HALO + 8, 128), F32)
    v1_s[:, BS:BS + HALO + 8, :] = jnp.zeros((NT, HALO + 8, 128), F32)
    kvs, carry_rows = {}, None
    for p, (kind, t) in enumerate(
            [("KV", 0), ("KV", 1), ("KV", 2), ("M", 0), ("KV", 3), ("M", 1),
             ("KV", 4), ("M", 2), ("M", 3), ("M", 4)]):
        lo, hi = _BANDS[t]
        if kind == "KV":
            res = _dot(bf16_rows(g_s, lo, hi), wraw[R_VB, :, _lane(t)])
            rh = _head_of(lax.broadcasted_iota(jnp.int32, res.shape, 0) + lo)
            ch = _head_of(lax.broadcasted_iota(jnp.int32, res.shape, 1) + 128 * t)
            kvs[t] = jnp.where(rh == ch, res, 0.0).astype(BF16)
        else:
            res = _dot(kvs[t], wraw[R_OB, 128 * t:128 * (t + 1), :])
            done = res
            if t:
                n = _BANDS[t - 1][1] - lo
                done = jnp.concatenate([res[0:n] + carry_rows, res[n:]], axis=0)
            end = _BANDS[t + 1][0] if t + 1 < NT else hi
            carry_rows = res[end - lo:]
            done = _pack(done[0:end - lo].astype(BF16))
            for c in range(NT):
                tu[P_M, c, lo // 2:end // 2, :] = done[:, _lane(c)]
        run_tasks({0: [z_stage1], 3: [z_stage2]}.get(p, []), res)

    def rows_of(g):
        return 16 * (g // 2) + g % 2

    def lin_group(par, g, tok):
        rows = pl.ds(rows_of(g), 8, stride=2)
        pq = [_phi(gate(tok, qb_s[t, rows, :])) for t in range(NT)]
        den = _tree(jnp.add, [pq[t] * zrow[:, _lane(t)] for t in range(NT)])
        rec = _recip(_group_sum(den) + 1e-6)
        for t in range(NT):
            ab[par][t, rows, :] = pq[t] * rec

    def att_group(par, row0, g, tok):
        s0 = rows_of(g)

        def tap(t, w):
            return pl.ds(SKEW[t] + HALO + s0 - DIL * w, 8, stride=2)

        cvec = gate(tok, jnp.full((8, 128), EXP2_C, F32))
        qq = [q_s[t, pl.ds(s0, 8, stride=2), :] * cvec for t in range(NT)]
        logits = []
        for w in range(WIN):
            p = _tree(jnp.add, [qq[t] * kb[par][t, tap(t, w), :] for t in range(NT)])
            p = _group_sum(p)
            if par == 0 and s0 < DIL * w:
                pos = 2 * lax.broadcasted_iota(jnp.int32, p.shape, 0) + (s0 + row0)
                p = jnp.where(pos >= DIL * w, p, NEG)
            logits.append(p)
        m = _tree(jnp.maximum, logits)
        e = [jnp.exp2(logits[w] - m) for w in range(WIN)]
        rec = _recip(_tree(jnp.add, e))
        for t in range(NT):
            acc = _tree(jnp.add, [e[w] * vb[par][t, tap(t, w), :] for w in range(WIN)])
            ob[par][t, pl.ds(s0, 8, stride=2), :] = acc * rec

    def pair(j, carry):
        set_zero(j)
        row0 = 2 * BS * j
        tasks = collections.defaultdict(list)
        for c in range(NT):
            tasks[c] += [functools.partial(p_stage, P_M, c, half) for half in range(2)]
        for fn, lo, hi in ((functools.partial(lin_group, 0), 5, 17),
                           (functools.partial(att_group, 0, row0), 20, 32),
                           (functools.partial(lin_group, 1), 33, 39),
                           (functools.partial(att_group, 1, row0), 40, 52)):
            for g, p in enumerate(_spread(NG, lo, hi)):
                tasks[p].append(functools.partial(fn, g))

        lhs = {}
        p = 0
        for kind, par in (("Bq", 0), ("K", 0), ("V", 0), ("Q", 0),
                          ("K", 1), ("Bq", 1), ("V", 1), ("Q", 1),
                          ("Bo", 0), ("Ao", 0), ("Bo", 1), ("Ao", 1)):
            blk = 2 * j + par
            rows = pl.ds(pl.multiple_of(blk * BS, BS), BS)
            src = {"Bq": "xb", "Bo": "a", "Ao": "o"}.get(kind, "xa")
            if (src, par) not in lhs:
                if src in ("xa", "xb"):
                    lhs[src, par] = (xa if src == "xa" else xb)[rows, :]
                else:
                    lhs[src, par] = bf16_rows((ab if src == "a" else ob)[par], 0, BS)
            x = lhs[src, par]
            for t in range(NT):
                halo = pl.ds(SKEW[t], HALO)
                body = pl.ds(SKEW[t] + HALO, BS)
                tail = pl.ds(SKEW[t] + BS, HALO)
                if kind in ("Bo", "Ao"):
                    slot, col0 = (P_M, D) if kind == "Bo" else (P_OA, 0)
                    res = _dot(x, _unpack(wp[slot, :, _lane(t)]))
                    out_s[rows, col0 + 128 * t:col0 + 128 * (t + 1)] = res.astype(BF16)
                    if (kind, par) == ("Ao", 0) and t == NT - 1:
                        out_copy(blk, 0, 2 * D).start()
                    elif (kind, par) == ("Bo", 1) and t == NT - 1:
                        out_copy(blk, D, D).start()
                    elif (kind, par) == ("Ao", 1) and t >= 2:
                        (out_copy(blk, 0, 384) if t == 2
                         else out_copy(blk, 128 * t, 128)).start()
                else:
                    slot = {"Q": P_QA, "K": P_KA, "V": P_VA, "Bq": P_QB}[kind]
                    if kind == "K":
                        kb[par][t, halo, :] = kb[1 - par][t, tail, :]
                    if kind == "V":
                        prev = vb[1 - par][t, tail, :]
                    if p == 0:
                        res = _dot(x, _unpack(wq0[...]))
                    else:
                        res = _dot_nt(x, _unpack(wp[slot, 64 * t:64 * (t + 1), :]))
                    if kind == "Q":
                        q_s[t, 0:BS, :] = res
                    elif kind == "Bq":
                        qb_s[t, 0:BS, :] = res
                    elif kind == "K":
                        kb[par][t, body, :] = res
                    else:
                        vb[par][t, body, :] = res
                        if par == 0:
                            prev = jnp.where(
                                j == 0, jnp.broadcast_to(res[0:1, :], (HALO, 128)), prev)
                        vb[par][t, halo, :] = prev
                run_tasks(tasks[p], res)
                p += 1
        return carry

    lax.fori_loop(0, NB // 2, pair, 0)
    pltpu.make_async_copy(out_s, out_hbm, sems.at[0]).wait()


@jax.jit
def pallas_concat_heads__sliding_local_dilated__linear_attn_block__prompt_kernel(
    A_x: jax.Array,
    A_wqkv: jax.Array,
    A_wo: jax.Array,
    B_x: jax.Array,
    B_wqkv: jax.Array,
    B_wo: jax.Array,
):
    any_spec = pl.BlockSpec(memory_space=pl.ANY)
    slab = lambda rows: pltpu.VMEM((NT, rows + PAD, 128), F32)
    extra = {name: True for name in ("disable_bounds_checks", "disable_semaphore_checks")
             if hasattr(pltpu.CompilerParams, name)}
    out = pl.pallas_call(
        _kernel,
        out_shape=jax.ShapeDtypeStruct((S, 2 * D), BF16),
        in_specs=[any_spec] * 6,
        out_specs=any_spec,
        scratch_shapes=[
            pltpu.VMEM((S, D), BF16),
            pltpu.VMEM((S, D), BF16),
            pltpu.VMEM((8, D, D), BF16),
            pltpu.VMEM((6, D // 2, D), U32),
            pltpu.VMEM((D // 2, 128), U32),
            pltpu.VMEM((D // 2, D), U32),
            pltpu.VMEM((6, NT, D // 2, 128), U32),
            pltpu.VMEM((NT, D, 128), F32),
            pltpu.VMEM((D // 2, SEG), U32),
            pltpu.VMEM((D, 128), F32),
            pltpu.VMEM((D, 128), F32),
            pltpu.VMEM((8, D), F32),
            slab(BS),
            slab(HALO + BS), slab(HALO + BS),
            slab(HALO + BS), slab(HALO + BS),
            slab(BS),
            slab(BS), slab(BS),
            slab(BS), slab(BS),
            pltpu.VMEM((S, 2 * D), BF16),
            pltpu.SemaphoreType.DMA((3,)),
        ],
        compiler_params=pltpu.CompilerParams(
            vmem_limit_bytes=64 * 1024 * 1024, **extra),
    )(A_x.reshape(S, D), A_wqkv, A_wo, B_x.reshape(S, D), B_wqkv, B_wo)
    return out.reshape(1, S, 2 * D)
```

```python
import collections
import functools
import math

import jax
import jax.numpy as jnp
from jax import lax
import jax.experimental.pallas as pl
import jax.experimental.pallas.tpu as pltpu

S = 2048
D = 640
H = 32
DH = D // H
NT = D // 128
WIN = 8
DIL = 2
HALO = 16
SEG0 = 256
SEG = (S - SEG0) // 2
SEGS = (0, SEG0, SEG0 + SEG, S)
BS = 256
NB = S // BS
NG = BS // 8
PAD = 24
SKEW = (0, 1, 0, 1, 0)

F32 = jnp.float32
BF16 = jnp.bfloat16
U32 = jnp.uint32
LOG2E = math.log2(math.e)
EXP2_C = DH ** -0.5 * LOG2E
NEG = -1e9 * LOG2E

R_KB, R_QA, R_KA, R_VA, R_QB, R_VB, R_OB, R_OA = range(8)
P_QA, P_KA, P_VA, P_QB, P_OA, P_M = range(6)

_BANDS = [(((128 * j) // DH * DH) // 16 * 16,
           -((-((128 * j + 127) // DH + 1) * DH) // 16) * 16) for j in range(NT)]


def _dot(a, b):
    return jnp.dot(a, b, preferred_element_type=F32)


def _dot_nt(a, b):
    return lax.dot_general(a, b, (((1,), (1,)), ((), ())), preferred_element_type=F32)


def _phi(t):
    return jnp.where(t > 0, t + 1.0, jnp.exp(t)) + 1e-6


def _recip(x):
    r = pl.reciprocal(x, approx=True)
    return r * (2.0 - x * r)


def _tree(fn, xs):
    xs = list(xs)
    while len(xs) > 1:
        xs = [fn(xs[j], xs[j + 1]) if j + 1 < len(xs) else xs[j]
              for j in range(0, len(xs), 2)]
    return xs[0]


def _group_sum(p):
    p = p + pltpu.roll(p, 64, 1)
    return p + pltpu.roll(p, 32, 1)


def _lane(t):
    return slice(128 * t, 128 * (t + 1))


def _unpack(u):
    return pltpu.bitcast(u, BF16)


def _pack(b):
    return pltpu.bitcast(b, U32)


def _head_of(x):
    return lax.shift_right_logical(x * 3277, 16)


def _spread(n, lo, hi):
    return [lo + (j * (hi - lo + 1)) // n for j in range(n)]


def _kernel(xa_hbm, wa_hbm, woa_hbm, xb_hbm, wb_hbm, wob_hbm, out_hbm,
            xa, xb, wraw, wp, wq0, wkT, tu, g_s, pk_u, zacc, ztmp, zrow,
            q_s, k0_s, k1_s, v0_s, v1_s, qb_s, o0_s, o1_s, a0_s, a1_s, out_s,
            sems):
    kb, vb, ob, ab = (k0_s, k1_s), (v0_s, v1_s), (o0_s, o1_s), (a0_s, a1_s)

    w_src = {
        R_QA: wa_hbm.at[:, 0:D], R_KA: wa_hbm.at[:, D:2 * D],
        R_VA: wa_hbm.at[:, 2 * D:3 * D], R_QB: wb_hbm.at[:, 0:D],
        R_VB: wb_hbm.at[:, 2 * D:3 * D], R_OB: wob_hbm, R_OA: woa_hbm,
    }

    def wk_copy(j):
        rows = pl.ds(128 * j, 128)
        return pltpu.make_async_copy(
            wb_hbm.at[rows, pl.ds(D, D)], wraw.at[R_KB, rows], sems.at[j // 3])

    def w_copy(i):
        sem = sems.at[2 if i in (R_VB, R_OB) else 1]
        return pltpu.make_async_copy(w_src[i], wraw.at[i], sem)

    def xb_copy(s):
        rows = pl.ds(SEGS[s], SEGS[s + 1] - SEGS[s])
        return pltpu.make_async_copy(xb_hbm.at[rows], xb.at[rows], sems.at[(2, 0, 1)[s]])

    def xa_copy():
        return pltpu.make_async_copy(xa_hbm, xa, sems.at[2])

    def out_copy(i, col0, ncol):
        rows, cols = pl.ds(i * BS, BS), pl.ds(col0, ncol)
        return pltpu.make_async_copy(out_s.at[rows, cols], out_hbm.at[rows, cols],
                                     sems.at[0])

    zero = [None]

    def set_zero(i):
        zero[0] = lax.shift_right_logical(i, 8)

    def gate(tok, x):
        reps = (x.shape[0] // 8, x.shape[1] // 128)
        if tok.dtype != x.dtype:
            tok = pltpu.bitcast(tok, x.dtype)
        if reps[1] > 1:
            tok = jnp.concatenate([tok] * reps[1], axis=1)
        if reps[0] > 1:
            tok = jnp.concatenate([tok] * reps[0], axis=0)
        never = jnp.full(x.shape, zero[0], jnp.int32) != 0
        return jnp.where(never, tok, x)

    def run_tasks(tasks, res):
        n = len(tasks)
        for j, fn in enumerate(tasks):
            row = (res.shape[0] * j // n) // 8 * 8
            fn(res[row:row + 8, 0:128])

    def t_stage(slot, raw, j, tok):
        slab = _unpack(gate(tok, _pack(wraw[raw, 128 * j:128 * (j + 1), :])))
        tu[slot, j, 0:D // 2, :] = _pack(slab.T)

    def c_stage(slot, raw, j, tok):
        tu[slot, j, 0:D // 2, :] = gate(tok, _pack(wraw[raw, :, _lane(j)]))

    def p_stage(slot, j, half, tok):
        for e in range(half * DH // 4, (half + 1) * DH // 4):
            lo = gate(tok, tu[slot, j, pl.ds(e, H // 2, stride=DH // 2), :])
            hi = tu[slot, j, pl.ds(e + D // 4, H // 2, stride=DH // 2), :]
            wp[slot, 32 * e:32 * e + 16, _lane(j)] = (lo & 0xFFFF) | (hi << 16)
            wp[slot, 32 * e + 16:32 * e + 32, _lane(j)] = (
                (lo >> 16) | (hi & jnp.uint32(0xFFFF0000)))

    def n_stage(tok):
        wq0[...] = _pack(_unpack(gate(tok, wp[P_QB, 0:64, :])).T)

    def z_stage1(tok):
        for d in range(DH):
            for b in range(2):
                ztmp[pl.ds(H * d + b, H // 2, stride=2), :] = gate(
                    tok, zacc[pl.ds(d + b * D // 2, H // 2, stride=DH), :])

    def z_stage2(tok):
        for t in range(NT):
            zt = gate(tok, ztmp[128 * t:128 * (t + 1), :]).T
            zt = jnp.sum(zt, axis=0, keepdims=True)
            zrow[:, _lane(t)] = jnp.broadcast_to(zt, (8, 128))

    for j in range(NT):
        wk_copy(j).start()
    xb_copy(0).start()
    for group in ((0, 1, 2), (3, 4)):
        for j in group:
            wk_copy(j).wait()
        for j in group:
            wkT[:, _lane(j)] = _pack(wraw[R_KB, 128 * j:128 * (j + 1), :].T)

    def stats(lo, nrows, init, tasks):
        p = 0
        wk_val = _unpack(wkT[...])
        for n in range(nrows // 128):
            if n == 0:
                res = _dot(xb[pl.ds(lo, 128), :], wraw[R_KB])
                pk = _phi(res).T
            else:
                res = _dot_nt(wk_val, xb[pl.ds(lo + 128 * n, 128), :])
                pk = _phi(res)
            if init and n == 0:
                zacc[0:D, :] = pk
            else:
                zacc[0:D, :] += pk
            pk_u[:, _lane(n)] = _pack(pk.astype(BF16))
            run_tasks(tasks[p], res)
            p += 1
        for k0, kn in (((0, 128), (128, nrows - 128)) if init else ((0, nrows),)):
            pk_val = _unpack(pk_u[:, k0:k0 + kn])
            for c in range(NT):
                res = _dot(pk_val, xb[pl.ds(lo + k0, kn), _lane(c)])
                if init and k0 == 0:
                    g_s[c] = res
                else:
                    g_s[c] += res
                run_tasks(tasks[p], res[0:512] if c == NT - 1 else res)
                p += 1

    xb_copy(0).wait()
    xb_copy(1).start()
    xb_copy(2).start()
    for i in (R_QB, R_KA):
        w_copy(i).start()
    stats(0, SEG0, True, collections.defaultdict(list))

    prep = ((P_QB, R_QB), (P_KA, R_KA), (P_VA, R_VA), (P_QA, R_QA), (P_OA, R_OA))

    def stats_step(it, carry):
        @pl.when(it == 0)
        def _():
            for i in (R_VA, R_QA, R_OA):
                w_copy(i).start()
            xb_copy(1).wait()

        @pl.when(it == 1)
        def _():
            for i in (R_VB, R_OB):
                w_copy(i).start()
            xa_copy().start()
            xb_copy(2).wait()
            for _, raw in prep:
                w_copy(raw).wait()

        set_zero(it)
        todo = [functools.partial(c_stage if slot == P_OA else t_stage, slot,
                                  it * raw + (1 - it) * R_KB, j)
                for slot, raw in prep for j in range(NT)]
        todo += [functools.partial(p_stage, slot, j, half)
                 for slot, _ in prep for j in range(NT) for half in range(2)]
        todo.insert(len(todo) - 20, n_stage)
        tasks = collections.defaultdict(list)
        room = [1.0] * (SEG // 128) + [1.5] * NT
        for n, fn in enumerate(todo):
            x, p = (n + 0.5) * sum(room) / len(todo), 0
            while x > room[p]:
                x -= room[p]
                p += 1
            tasks[p].append(fn)
        stats(pl.multiple_of(SEG0 + it * SEG, 128), SEG, False, tasks)
        return carry + it

    set_zero(lax.fori_loop(0, 2, stats_step, 0))

    for i in (R_VB, R_OB):
        w_copy(i).wait()
    xa_copy().wait()

    def bf16_rows(src, lo, hi):
        return jnp.concatenate([src[t, lo:hi, :] for t in range(NT)], axis=1).astype(BF16)

    k1_s[:, BS:BS + HALO + 8, :] = jnp.zeros((NT, HALO + 8, 128), F32)
    v1_s[:, BS:BS + HALO + 8, :] = jnp.zeros((NT, HALO + 8, 128), F32)
    kvs, carry_rows = {}, None
    for p, (kind, t) in enumerate(
            [("KV", 0), ("KV", 1), ("KV", 2), ("M", 0), ("KV", 3), ("M", 1),
             ("KV", 4), ("M", 2), ("M", 3), ("M", 4)]):
        lo, hi = _BANDS[t]
        if kind == "KV":
            res = _dot(bf16_rows(g_s, lo, hi), wraw[R_VB, :, _lane(t)])
            rh = _head_of(lax.broadcasted_iota(jnp.int32, res.shape, 0) + lo)
            ch = _head_of(lax.broadcasted_iota(jnp.int32, res.shape, 1) + 128 * t)
            kvs[t] = jnp.where(rh == ch, res, 0.0).astype(BF16)
        else:
            res = _dot(kvs[t], wraw[R_OB, 128 * t:128 * (t + 1), :])
            done = res
            if t:
                n = _BANDS[t - 1][1] - lo
                done = jnp.concatenate([res[0:n] + carry_rows, res[n:]], axis=0)
            end = _BANDS[t + 1][0] if t + 1 < NT else hi
            carry_rows = res[end - lo:] if end < hi else None
            done = _pack(done[0:end - lo].astype(BF16))
            for c in range(NT):
                tu[P_M, c, lo // 2:end // 2, :] = done[:, _lane(c)]
        run_tasks({0: [z_stage1], 3: [z_stage2]}.get(p, []), res)

    def rows_of(g):
        return 16 * (g // 2) + g % 2

    def lin_group(par, g, tok):
        rows = pl.ds(rows_of(g), 8, stride=2)
        pq = [_phi(gate(tok, qb_s[t, rows, :])) for t in range(NT)]
        den = _tree(jnp.add, [pq[t] * zrow[:, _lane(t)] for t in range(NT)])
        rec = _recip(_group_sum(den) + 1e-6)
        for t in range(NT):
            ab[par][t, rows, :] = pq[t] * rec

    def att_group(par, row0, g, tok):
        s0 = rows_of(g)

        def tap(t, w):
            return pl.ds(SKEW[t] + HALO + s0 - DIL * w, 8, stride=2)

        cvec = gate(tok, jnp.full((8, 128), EXP2_C, F32))
        qq = [q_s[t, pl.ds(s0, 8, stride=2), :] * cvec for t in range(NT)]
        logits = []
        for w in range(WIN):
            p = _tree(jnp.add, [qq[t] * kb[par][t, tap(t, w), :] for t in range(NT)])
            p = _group_sum(p)
            if par == 0 and s0 < DIL * w:
                pos = 2 * lax.broadcasted_iota(jnp.int32, p.shape, 0) + (s0 + row0)
                p = jnp.where(pos >= DIL * w, p, NEG)
            logits.append(p)
        m = _tree(jnp.maximum, logits)
        e = [jnp.exp2(logits[w] - m) for w in range(WIN)]
        rec = _recip(_tree(jnp.add, e))
        for t in range(NT):
            acc = _tree(jnp.add, [e[w] * vb[par][t, tap(t, w), :] for w in range(WIN)])
            ob[par][t, pl.ds(s0, 8, stride=2), :] = acc * rec

    def pair(j, carry):
        set_zero(j)
        row0 = 2 * BS * j
        tasks = collections.defaultdict(list)
        for c in range(NT):
            tasks[c] += [functools.partial(p_stage, P_M, c, half) for half in range(2)]
        for fn, lo, hi in ((functools.partial(lin_group, 0), 5, 17),
                           (functools.partial(att_group, 0, row0), 20, 32),
                           (functools.partial(lin_group, 1), 33, 39),
                           (functools.partial(att_group, 1, row0), 40, 52)):
            for g, p in enumerate(_spread(NG, lo, hi)):
                tasks[p].append(functools.partial(fn, g))

        lhs = {}
        p = 0
        for kind, par in (("Bq", 0), ("K", 0), ("V", 0), ("Q", 0),
                          ("K", 1), ("Bq", 1), ("V", 1), ("Q", 1),
                          ("Bo", 0), ("Ao", 0), ("Bo", 1), ("Ao", 1)):
            blk = 2 * j + par
            rows = pl.ds(pl.multiple_of(blk * BS, BS), BS)
            src = {"Bq": "xb", "Bo": "a", "Ao": "o"}.get(kind, "xa")
            if (src, par) not in lhs:
                if src in ("xa", "xb"):
                    lhs[src, par] = (xa if src == "xa" else xb)[rows, :]
                else:
                    lhs[src, par] = bf16_rows((ab if src == "a" else ob)[par], 0, BS)
            x = lhs[src, par]
            for t in range(NT):
                halo = pl.ds(SKEW[t], HALO)
                body = pl.ds(SKEW[t] + HALO, BS)
                tail = pl.ds(SKEW[t] + BS, HALO)
                if kind in ("Bo", "Ao"):
                    slot, col0 = (P_M, D) if kind == "Bo" else (P_OA, 0)
                    res = _dot(x, _unpack(wp[slot, :, _lane(t)]))
                    out_s[rows, col0 + 128 * t:col0 + 128 * (t + 1)] = res.astype(BF16)
                    if (kind, par) == ("Ao", 0) and t == NT - 1:
                        out_copy(blk, 0, 2 * D).start()
                    elif (kind, par) == ("Bo", 1) and t == NT - 1:
                        out_copy(blk, D, D).start()
                    elif (kind, par) == ("Ao", 1) and t >= 2:
                        (out_copy(blk, 0, 384) if t == 2
                         else out_copy(blk, 128 * t, 128)).start()
                else:
                    slot = {"Q": P_QA, "K": P_KA, "V": P_VA, "Bq": P_QB}[kind]
                    if kind == "K":
                        kb[par][t, halo, :] = kb[1 - par][t, tail, :]
                    if kind == "V":
                        prev = vb[1 - par][t, tail, :]
                    if p == 0:
                        res = _dot(x, _unpack(wq0[...]))
                    else:
                        res = _dot_nt(x, _unpack(wp[slot, 64 * t:64 * (t + 1), :]))
                    if kind == "Q":
                        q_s[t, 0:BS, :] = res
                    elif kind == "Bq":
                        qb_s[t, 0:BS, :] = res
                    elif kind == "K":
                        kb[par][t, body, :] = res
                    else:
                        vb[par][t, body, :] = res
                        if par == 0:
                            prev = jnp.where(
                                j == 0, jnp.broadcast_to(res[0:1, :], (HALO, 128)), prev)
                        vb[par][t, halo, :] = prev
                run_tasks(tasks[p], res)
                p += 1
        return carry

    lax.fori_loop(0, NB // 2, pair, 0)
    pltpu.make_async_copy(out_s, out_hbm, sems.at[0]).wait()


@jax.jit
def pallas_concat_heads__sliding_local_dilated__linear_attn_block__prompt_kernel(
    A_x: jax.Array,
    A_wqkv: jax.Array,
    A_wo: jax.Array,
    B_x: jax.Array,
    B_wqkv: jax.Array,
    B_wo: jax.Array,
):
    any_spec = pl.BlockSpec(memory_space=pl.ANY)
    slab = lambda rows: pltpu.VMEM((NT, rows + PAD, 128), F32)
    extra = {name: True for name in ("disable_bounds_checks", "disable_semaphore_checks")
             if hasattr(pltpu.CompilerParams, name)}
    out = pl.pallas_call(
        _kernel,
        out_shape=jax.ShapeDtypeStruct((S, 2 * D), BF16),
        in_specs=[any_spec] * 6,
        out_specs=any_spec,
        scratch_shapes=[
            pltpu.VMEM((S, D), BF16),
            pltpu.VMEM((S, D), BF16),
            pltpu.VMEM((8, D, D), BF16),
            pltpu.VMEM((6, D // 2, D), U32),
            pltpu.VMEM((D // 2, 128), U32),
            pltpu.VMEM((D // 2, D), U32),
            pltpu.VMEM((6, NT, D // 2 + 16, 128), U32),
            pltpu.VMEM((NT, D, 128), F32),
            pltpu.VMEM((D // 2, SEG), U32),
            pltpu.VMEM((D + PAD, 128), F32),
            pltpu.VMEM((D + 8, 128), F32),
            pltpu.VMEM((8, D), F32),
            slab(BS),
            slab(HALO + BS), slab(HALO + BS),
            slab(HALO + BS), slab(HALO + BS),
            slab(BS),
            slab(BS), slab(BS),
            slab(BS), slab(BS),
            pltpu.VMEM((S, 2 * D), BF16),
            pltpu.SemaphoreType.DMA((3,)),
        ],
        compiler_params=pltpu.CompilerParams(
            vmem_limit_bytes=64 * 1024 * 1024, **extra),
    )(A_x.reshape(S, D), A_wqkv, A_wo, B_x.reshape(S, D), B_wqkv, B_wo)
    return out.reshape(1, S, 2 * D)
```

```python
import collections
import functools
import math

import jax
import jax.numpy as jnp
from jax import lax
import jax.experimental.pallas as pl
import jax.experimental.pallas.tpu as pltpu

S = 2048
D = 640
H = 32
DH = D // H
NT = D // 128
WIN = 8
DIL = 2
HALO = 16
SEG0 = 256
SEG = (S - SEG0) // 2
SEGS = (0, SEG0, SEG0 + SEG, S)
F0 = 256
BS = 256
NB = S // BS
NG = BS // 8
PAD = 24
SKEW = (0, 1, 0, 1, 0)

F32 = jnp.float32
BF16 = jnp.bfloat16
U32 = jnp.uint32
LOG2E = math.log2(math.e)
EXP2_C = DH ** -0.5 * LOG2E
NEG = -1e9 * LOG2E

R_KB, R_QA, R_KA, R_VA, R_QB, R_VB, R_OB, R_OA = range(8)
P_QA, P_KA, P_VA, P_QB, P_OA, P_M = range(6)

_BANDS = [(((128 * j) // DH * DH) // 16 * 16,
           -((-((128 * j + 127) // DH + 1) * DH) // 16) * 16) for j in range(NT)]


def _dot(a, b):
    return jnp.dot(a, b, preferred_element_type=F32)


def _dot_nt(a, b):
    return lax.dot_general(a, b, (((1,), (1,)), ((), ())), preferred_element_type=F32)


def _phi(t):
    return jnp.where(t > 0, t + 1.0, jnp.exp(t)) + 1e-6


def _recip(x):
    r = pl.reciprocal(x, approx=True)
    return r * (2.0 - x * r)


def _tree(fn, xs):
    xs = list(xs)
    while len(xs) > 1:
        xs = [fn(xs[j], xs[j + 1]) if j + 1 < len(xs) else xs[j]
              for j in range(0, len(xs), 2)]
    return xs[0]


def _group_sum(p):
    p = p + pltpu.roll(p, 64, 1)
    return p + pltpu.roll(p, 32, 1)


def _lane(t):
    return slice(128 * t, 128 * (t + 1))


def _unpack(u):
    return pltpu.bitcast(u, BF16)


def _pack(b):
    return pltpu.bitcast(b, U32)


def _head_of(x):
    return lax.shift_right_logical(x * 3277, 16)


def _spread(n, lo, hi):
    return [lo + (j * (hi - lo + 1)) // n for j in range(n)]


def _kernel(xa_hbm, wa_hbm, woa_hbm, xb_hbm, wb_hbm, wob_hbm, out_hbm,
            xa, xb, wraw, wp, wq0, wkT, tu, g_s, pk_u, zacc, ztmp, zrow,
            q_s, k0_s, k1_s, v0_s, v1_s, qb_s, o0_s, o1_s, a0_s, a1_s, out_s,
            sems):
    kb, vb, ob, ab = (k0_s, k1_s), (v0_s, v1_s), (o0_s, o1_s), (a0_s, a1_s)

    w_src = {
        R_QA: wa_hbm.at[:, 0:D], R_KA: wa_hbm.at[:, D:2 * D],
        R_VA: wa_hbm.at[:, 2 * D:3 * D], R_QB: wb_hbm.at[:, 0:D],
        R_VB: wb_hbm.at[:, 2 * D:3 * D], R_OB: wob_hbm, R_OA: woa_hbm,
    }

    def wk_copy(part):
        lo, hi = ((0, F0), (F0, D))[part]
        return pltpu.make_async_copy(
            wb_hbm.at[:, pl.ds(D + lo, hi - lo)], wraw.at[R_KB, :, pl.ds(lo, hi - lo)],
            sems.at[part])

    def x0_copy(h):
        r0 = 128 * h if isinstance(h, int) else pl.multiple_of(128 * h, 128)
        rows = pl.ds(r0, 128)
        return pltpu.make_async_copy(xb_hbm.at[rows], xb.at[rows], sems.at[2])

    def w_copy(i):
        sem = sems.at[2 if i in (R_VB, R_OB) else 1]
        return pltpu.make_async_copy(w_src[i], wraw.at[i], sem)

    def xb_copy(s):
        rows = pl.ds(SEGS[s], SEGS[s + 1] - SEGS[s])
        return pltpu.make_async_copy(xb_hbm.at[rows], xb.at[rows], sems.at[s - 1])

    def xa_copy():
        return pltpu.make_async_copy(xa_hbm, xa, sems.at[2])

    def out_copy(i, col0, ncol):
        rows, cols = pl.ds(i * BS, BS), pl.ds(col0, ncol)
        return pltpu.make_async_copy(out_s.at[rows, cols], out_hbm.at[rows, cols],
                                     sems.at[0])

    zero = [None]

    def set_zero(i):
        zero[0] = lax.shift_right_logical(i, 8)

    def gate(tok, x):
        reps = (x.shape[0] // 8, x.shape[1] // 128)
        if tok.dtype != x.dtype:
            tok = pltpu.bitcast(tok, x.dtype)
        if reps[1] > 1:
            tok = jnp.concatenate([tok] * reps[1], axis=1)
        if reps[0] > 1:
            tok = jnp.concatenate([tok] * reps[0], axis=0)
        never = jnp.full(x.shape, zero[0], jnp.int32) != 0
        return jnp.where(never, tok, x)

    def run_tasks(tasks, res):
        n = len(tasks)
        for j, fn in enumerate(tasks):
            row = (res.shape[0] * j // n) // 8 * 8
            fn(res[row:row + 8, 0:128])

    def t_stage(slot, raw, j, tok):
        slab = _unpack(gate(tok, _pack(wraw[raw, 128 * j:128 * (j + 1), :])))
        tu[slot, j, 0:D // 2, :] = _pack(slab.T)

    def c_stage(slot, raw, j, tok):
        tu[slot, j, 0:D // 2, :] = gate(tok, _pack(wraw[raw, :, _lane(j)]))

    def p_stage(slot, j, half, tok):
        for e in range(half * DH // 4, (half + 1) * DH // 4):
            lo = gate(tok, tu[slot, j, pl.ds(e, H // 2, stride=DH // 2), :])
            hi = tu[slot, j, pl.ds(e + D // 4, H // 2, stride=DH // 2), :]
            wp[slot, 32 * e:32 * e + 16, _lane(j)] = (lo & 0xFFFF) | (hi << 16)
            wp[slot, 32 * e + 16:32 * e + 32, _lane(j)] = (
                (lo >> 16) | (hi & jnp.uint32(0xFFFF0000)))

    def n_stage(tok):
        wq0[...] = _pack(_unpack(gate(tok, wp[P_QB, 0:64, :])).T)

    def z_stage1(tok):
        for d in range(DH):
            for b in range(2):
                ztmp[pl.ds(H * d + b, H // 2, stride=2), :] = gate(
                    tok, zacc[pl.ds(d + b * D // 2, H // 2, stride=DH), :])

    def z_stage2(tok):
        for t in range(NT):
            zt = gate(tok, ztmp[128 * t:128 * (t + 1), :]).T
            zt = jnp.sum(zt, axis=0, keepdims=True)
            zrow[:, _lane(t)] = jnp.broadcast_to(zt, (8, 128))

    def stats(lo, nrows, tasks):
        p = 0
        wk_val = _unpack(wkT[...])
        for n in range(nrows // 128):
            if n == 0:
                res = _dot(xb[pl.ds(lo, 128), :], wraw[R_KB])
                pk = _phi(res).T
            else:
                res = _dot_nt(wk_val, xb[pl.ds(lo + 128 * n, 128), :])
                pk = _phi(res)
            zacc[0:D, :] += pk
            pk_u[:, _lane(n)] = _pack(pk.astype(BF16))
            run_tasks(tasks[p], res)
            p += 1
        pk_val = _unpack(pk_u[:, 0:nrows])
        for c in range(NT):
            res = _dot(pk_val, xb[pl.ds(lo, nrows), _lane(c)])
            g_s[c] += res
            run_tasks(tasks[p], res[0:512] if c == NT - 1 else res)
            p += 1

    def wkt_stage(j, tok):
        slab = _unpack(gate(tok, _pack(wraw[R_KB, 128 * j:128 * (j + 1), :])))
        wkT[:, _lane(j)] = _pack(slab.T)

    def first_rows(f0, f1, tasks):
        p = 0
        for h in range(SEG0 // 128):
            res = _dot(xb[128 * h:128 * (h + 1), :], wraw[R_KB, :, f0:f1])
            pk = _phi(res).T
            if h == 0:
                zacc[f0:f1, :] = pk
            else:
                zacc[f0:f1, :] += pk
            pk_u[f0 // 2:f1 // 2, _lane(h)] = _pack(pk.astype(BF16))
            run_tasks(tasks[p], res)
            p += 1
        for h in range(SEG0 // 128):
            for t in range(f0 // 128, f1 // 128):
                res = _dot(_unpack(pk_u[64 * t:64 * (t + 1), _lane(h)]),
                           xb[128 * h:128 * (h + 1), :])
                for c in range(NT):
                    if h == 0:
                        g_s[c, 128 * t:128 * (t + 1), :] = res[:, _lane(c)]
                    else:
                        g_s[c, 128 * t:128 * (t + 1), :] += res[:, _lane(c)]
                run_tasks(tasks[p], res)
                p += 1

    def x0_start(h, carry):
        x0_copy(h).start()
        return carry + h

    wk_copy(0).start()
    set_zero(lax.fori_loop(0, SEG0 // 128, x0_start, 0))
    wk_copy(1).start()
    wk_copy(0).wait()
    for h in range(SEG0 // 128):
        x0_copy(h).wait()
    xb_copy(1).start()
    first_rows(0, F0, collections.defaultdict(list))
    wk_copy(1).wait()
    xb_copy(2).start()
    for i in (R_QB, R_KA):
        w_copy(i).start()
    tasks = collections.defaultdict(list)
    for j in range(NT):
        tasks[j].append(functools.partial(wkt_stage, j))
    first_rows(F0, D, tasks)

    prep = ((P_QB, R_QB), (P_KA, R_KA), (P_VA, R_VA), (P_QA, R_QA), (P_OA, R_OA))

    def stats_step(it, carry):
        @pl.when(it == 0)
        def _():
            for i in (R_VA, R_QA, R_OA):
                w_copy(i).start()
            xb_copy(1).wait()

        @pl.when(it == 1)
        def _():
            for i in (R_VB, R_OB):
                w_copy(i).start()
            xa_copy().start()
            xb_copy(2).wait()
            for _, raw in prep:
                w_copy(raw).wait()

        set_zero(it)
        todo = [functools.partial(c_stage if slot == P_OA else t_stage, slot,
                                  it * raw + (1 - it) * R_KB, j)
                for slot, raw in prep for j in range(NT)]
        todo += [functools.partial(p_stage, slot, j, half)
                 for slot, _ in prep for j in range(NT) for half in range(2)]
        todo.insert(len(todo) - 20, n_stage)
        tasks = collections.defaultdict(list)
        room = [1.0] * (SEG // 128) + [1.5] * NT
        for n, fn in enumerate(todo):
            x, p = (n + 0.5) * sum(room) / len(todo), 0
            while x > room[p]:
                x -= room[p]
                p += 1
            tasks[p].append(fn)
        stats(pl.multiple_of(SEG0 + it * SEG, 128), SEG, tasks)
        return carry + it

    set_zero(lax.fori_loop(0, 2, stats_step, 0))

    for i in (R_VB, R_OB):
        w_copy(i).wait()
    xa_copy().wait()

    def bf16_rows(src, lo, hi):
        return jnp.concatenate([src[t, lo:hi, :] for t in range(NT)], axis=1).astype(BF16)

    k1_s[:, BS:BS + HALO + 8, :] = jnp.zeros((NT, HALO + 8, 128), F32)
    v1_s[:, BS:BS + HALO + 8, :] = jnp.zeros((NT, HALO + 8, 128), F32)
    kvs, carry_rows = {}, None
    for p, (kind, t) in enumerate(
            [("KV", 0), ("KV", 1), ("KV", 2), ("M", 0), ("KV", 3), ("M", 1),
             ("KV", 4), ("M", 2), ("M", 3), ("M", 4)]):
        lo, hi = _BANDS[t]
        if kind == "KV":
            res = _dot(bf16_rows(g_s, lo, hi), wraw[R_VB, :, _lane(t)])
            rh = _head_of(lax.broadcasted_iota(jnp.int32, res.shape, 0) + lo)
            ch = _head_of(lax.broadcasted_iota(jnp.int32, res.shape, 1) + 128 * t)
            kvs[t] = jnp.where(rh == ch, res, 0.0).astype(BF16)
        else:
            res = _dot(kvs[t], wraw[R_OB, 128 * t:128 * (t + 1), :])
            done = res
            if t:
                n = _BANDS[t - 1][1] - lo
                done = jnp.concatenate([res[0:n] + carry_rows, res[n:]], axis=0)
            end = _BANDS[t + 1][0] if t + 1 < NT else hi
            carry_rows = res[end - lo:] if end < hi else None
            done = _pack(done[0:end - lo].astype(BF16))
            for c in range(NT):
                tu[P_M, c, lo // 2:end // 2, :] = done[:, _lane(c)]
        run_tasks({0: [z_stage1], 3: [z_stage2]}.get(p, []), res)

    def rows_of(g):
        return 16 * (g // 2) + g % 2

    def lin_group(par, g, tok):
        rows = pl.ds(rows_of(g), 8, stride=2)
        pq = [_phi(gate(tok, qb_s[t, rows, :])) for t in range(NT)]
        den = _tree(jnp.add, [pq[t] * zrow[:, _lane(t)] for t in range(NT)])
        rec = _recip(_group_sum(den) + 1e-6)
        for t in range(NT):
            ab[par][t, rows, :] = pq[t] * rec

    def att_group(par, row0, g, tok):
        s0 = rows_of(g)

        def tap(t, w):
            return pl.ds(SKEW[t] + HALO + s0 - DIL * w, 8, stride=2)

        cvec = gate(tok, jnp.full((8, 128), EXP2_C, F32))
        qq = [q_s[t, pl.ds(s0, 8, stride=2), :] * cvec for t in range(NT)]
        logits = []
        for w in range(WIN):
            p = _tree(jnp.add, [qq[t] * kb[par][t, tap(t, w), :] for t in range(NT)])
            p = _group_sum(p)
            if par == 0 and s0 < DIL * w:
                pos = 2 * lax.broadcasted_iota(jnp.int32, p.shape, 0) + (s0 + row0)
                p = jnp.where(pos >= DIL * w, p, NEG)
            logits.append(p)
        m = _tree(jnp.maximum, logits)
        e = [jnp.exp2(logits[w] - m) for w in range(WIN)]
        rec = _recip(_tree(jnp.add, e))
        for t in range(NT):
            acc = _tree(jnp.add, [e[w] * vb[par][t, tap(t, w), :] for w in range(WIN)])
            ob[par][t, pl.ds(s0, 8, stride=2), :] = acc * rec

    def pair(j, carry):
        set_zero(j)
        row0 = 2 * BS * j
        tasks = collections.defaultdict(list)
        for c in range(NT):
            tasks[c] += [functools.partial(p_stage, P_M, c, half) for half in range(2)]
        for fn, lo, hi in ((functools.partial(lin_group, 0), 5, 17),
                           (functools.partial(att_group, 0, row0), 20, 32),
                           (functools.partial(lin_group, 1), 33, 39),
                           (functools.partial(att_group, 1, row0), 40, 52)):
            for g, p in enumerate(_spread(NG, lo, hi)):
                tasks[p].append(functools.partial(fn, g))

        lhs = {}
        p = 0
        for kind, par in (("Bq", 0), ("K", 0), ("V", 0), ("Q", 0),
                          ("K", 1), ("Bq", 1), ("V", 1), ("Q", 1),
                          ("Bo", 0), ("Ao", 0), ("Bo", 1), ("Ao", 1)):
            blk = 2 * j + par
            rows = pl.ds(pl.multiple_of(blk * BS, BS), BS)
            src = {"Bq": "xb", "Bo": "a", "Ao": "o"}.get(kind, "xa")
            if (src, par) not in lhs:
                if src in ("xa", "xb"):
                    lhs[src, par] = (xa if src == "xa" else xb)[rows, :]
                else:
                    lhs[src, par] = bf16_rows((ab if src == "a" else ob)[par], 0, BS)
            x = lhs[src, par]
            for t in range(NT):
                halo = pl.ds(SKEW[t], HALO)
                body = pl.ds(SKEW[t] + HALO, BS)
                tail = pl.ds(SKEW[t] + BS, HALO)
                if kind in ("Bo", "Ao"):
                    slot, col0 = (P_M, D) if kind == "Bo" else (P_OA, 0)
                    res = _dot(x, _unpack(wp[slot, :, _lane(t)]))
                    out_s[rows, col0 + 128 * t:col0 + 128 * (t + 1)] = res.astype(BF16)
                    if (kind, par) == ("Ao", 0) and t == NT - 1:
                        out_copy(blk, 0, 2 * D).start()
                    elif (kind, par) == ("Bo", 1) and t == NT - 1:
                        out_copy(blk, D, D).start()
                    elif (kind, par) == ("Ao", 1) and t >= 2:
                        (out_copy(blk, 0, 384) if t == 2
                         else out_copy(blk, 128 * t, 128)).start()
                else:
                    slot = {"Q": P_QA, "K": P_KA, "V": P_VA, "Bq": P_QB}[kind]
                    if kind == "K":
                        kb[par][t, halo, :] = kb[1 - par][t, tail, :]
                    if kind == "V":
                        prev = vb[1 - par][t, tail, :]
                    if p == 0:
                        res = _dot(x, _unpack(wq0[...]))
                    else:
                        res = _dot_nt(x, _unpack(wp[slot, 64 * t:64 * (t + 1), :]))
                    if kind == "Q":
                        q_s[t, 0:BS, :] = res
                    elif kind == "Bq":
                        qb_s[t, 0:BS, :] = res
                    elif kind == "K":
                        kb[par][t, body, :] = res
                    else:
                        vb[par][t, body, :] = res
                        if par == 0:
                            prev = jnp.where(
                                j == 0, jnp.broadcast_to(res[0:1, :], (HALO, 128)), prev)
                        vb[par][t, halo, :] = prev
                run_tasks(tasks[p], res)
                p += 1
        return carry

    lax.fori_loop(0, NB // 2, pair, 0)
    pltpu.make_async_copy(out_s, out_hbm, sems.at[0]).wait()


@jax.jit
def pallas_concat_heads__sliding_local_dilated__linear_attn_block__prompt_kernel(
    A_x: jax.Array,
    A_wqkv: jax.Array,
    A_wo: jax.Array,
    B_x: jax.Array,
    B_wqkv: jax.Array,
    B_wo: jax.Array,
):
    any_spec = pl.BlockSpec(memory_space=pl.ANY)
    slab = lambda rows: pltpu.VMEM((NT, rows + PAD, 128), F32)
    extra = {name: True for name in ("disable_bounds_checks", "disable_semaphore_checks")
             if hasattr(pltpu.CompilerParams, name)}
    out = pl.pallas_call(
        _kernel,
        out_shape=jax.ShapeDtypeStruct((S, 2 * D), BF16),
        in_specs=[any_spec] * 6,
        out_specs=any_spec,
        scratch_shapes=[
            pltpu.VMEM((S, D), BF16),
            pltpu.VMEM((S, D), BF16),
            pltpu.VMEM((8, D, D), BF16),
            pltpu.VMEM((6, D // 2, D), U32),
            pltpu.VMEM((D // 2, 128), U32),
            pltpu.VMEM((D // 2, D), U32),
            pltpu.VMEM((6, NT, D // 2 + 16, 128), U32),
            pltpu.VMEM((NT, D, 128), F32),
            pltpu.VMEM((D // 2, SEG), U32),
            pltpu.VMEM((D + PAD, 128), F32),
            pltpu.VMEM((D + 8, 128), F32),
            pltpu.VMEM((8, D), F32),
            slab(BS),
            slab(HALO + BS), slab(HALO + BS),
            slab(HALO + BS), slab(HALO + BS),
            slab(BS),
            slab(BS), slab(BS),
            slab(BS), slab(BS),
            pltpu.VMEM((S, 2 * D), BF16),
            pltpu.SemaphoreType.DMA((3,)),
        ],
        compiler_params=pltpu.CompilerParams(
            vmem_limit_bytes=64 * 1024 * 1024, **extra),
    )(A_x.reshape(S, D), A_wqkv, A_wo, B_x.reshape(S, D), B_wqkv, B_wo)
    return out.reshape(1, S, 2 * D)
```
